```python
import os as _os
_os.environ.setdefault("JAX_PLATFORMS", "cpu")
import jax
import jax.numpy as jnp

def _softmax(x, axis=-1):
    return jax.nn.softmax(x, axis=axis)
def _gelu(x):
    return jax.nn.gelu(x, approximate=True)
def _silu(x):
    return jax.nn.silu(x)
def _sigmoid(x):
    return jax.nn.sigmoid(x)
def _layernorm(x, axis=-1, eps=1e-5):
    m = jnp.mean(x, axis=axis, keepdims=True)
    v = jnp.var(x, axis=axis, keepdims=True)
    return (x - m) / jnp.sqrt(v + eps)
def _scatter_add(tgt, idx, src, axis=0):
    return tgt.at[idx].add(src)
def _segment_sum(src, seg, n):
    return jax.ops.segment_sum(src, seg, n)
class _Rng:
    def __init__(self, key):
        self._k = key
    def _next(self):
        self._k, sub = jax.random.split(self._k)
        return sub
    def normal(self, shape):
        return jax.random.normal(self._next(), shape, dtype=jnp.bfloat16)
    def randint(self, lo, hi, shape):
        return jax.random.randint(self._next(), shape, lo, hi, dtype=jnp.int32)
    def uniform(self, shape, lo=0.0, hi=1.0):
        return jax.random.uniform(self._next(), shape, jnp.bfloat16, lo, hi)
    def permutation(self, n):
        return jax.random.permutation(self._next(), n)


kernel_name = 'interleave_layers__ssm_conv_h3__geglu_ffn__prompt'

def setup_inputs():
    _rng = _Rng(jax.random.key(int.from_bytes(__import__("os").urandom(4), "little")))
    _w = (lambda a: (lambda t: t.astype(jnp.bfloat16) if jnp.issubdtype(t.dtype, jnp.floating) else t)(jnp.asarray(a)))
    def _A_setup():
        B, S, D = 1, 2048, 448
        ks = 4
        return {
            "q": _w((lambda *s: _rng.normal(s) * 0.05)(B, S, D)),
            "k": _w((lambda *s: _rng.normal(s) * 0.8)(B, S, D)),
            "v": _w((lambda *s: _rng.normal(s) * 0.8)(B, S, D)),
            "shift_k": _w((lambda *s: _rng.normal(s) * 0.8)(D, ks) * 0.5),
            "ssm_k": _w((lambda *s: _rng.normal(s) * 0.8)(D, S) * (1.0 / S ** 0.5)),
            "ssm_D": _w((lambda *s: _rng.normal(s) * 0.8)(D)),
        }
    _A_in = _A_setup()

    def _B_setup():
        B, S, D, F = 1, 2048, 448, 1792
        return {
            "x": _w((lambda *s: _rng.normal(s) * 0.05)(B, S, D)),
            "w_gate": _w((lambda *s: _rng.normal(s) * 0.1)(D, F)),
            "w_up": _w((lambda *s: _rng.normal(s) * 0.1)(D, F)),
            "w_down": _w((lambda *s: _rng.normal(s) * 0.1)(F, D)),
        }
    _B_in = _B_setup()

    return {
        "A_q": _A_in["q"],
        "A_k": _A_in["k"],
        "A_v": _A_in["v"],
        "A_shift_k": _A_in["shift_k"],
        "A_ssm_k": _A_in["ssm_k"],
        "A_ssm_D": _A_in["ssm_D"],
        "B_x": _B_in["x"],
        "B_w_gate": _B_in["w_gate"],
        "B_w_up": _B_in["w_up"],
        "B_w_down": _B_in["w_down"],
    }

def reference(A_q, A_k, A_v, A_shift_k, A_ssm_k, A_ssm_D, B_x, B_w_gate, B_w_up, B_w_down):
    def _A_ref(q, k, v, shift_k, ssm_k, ssm_D):
        B, S, D = q.shape
        ks = shift_k.shape[-1]
        k_pad = jnp.pad(k, ((0, 0), (ks - 1, 0), (0, 0)))
        k_shift = jnp.zeros_like(k)
        for t in range(ks):
            k_shift = k_shift + k_pad[:, t:t + S, :] * shift_k[:, ks - 1 - t][None, None, :]
        kv = k_shift * v
        L = 2 * S
        kv_pad = jnp.pad(kv, ((0, 0), (0, S), (0, 0)))
        kf_pad = jnp.pad(ssm_k, ((0, 0), (0, S)))
        kv_f = (lambda x, axes=(-2,-1): jnp.fft.rfft2(x.astype(jnp.float32), axes=axes))(kv_pad[:, None, :, :], axes=(1, 2))
        kf_f = (lambda x, axes=(-2,-1): jnp.fft.rfft2(x.astype(jnp.float32), axes=axes))(kf_pad[:, None, :], axes=(1, 2))
        kf_f = (lambda x, *d: x.transpose(*d))(kf_f, 1, 2, 0)
        y_f = kv_f * kf_f[None, :, :, :]
        y = (lambda x, s, axes=(-2,-1): jnp.fft.irfft2(x, s=s, axes=axes).astype(jnp.bfloat16))(y_f, (1, L), axes=(1, 2))[:, 0, :S, :]
        y = y + kv * ssm_D[None, None, :]
        return q * y

    def _B_ref(x, w_gate, w_up, w_down):
        return (_gelu(x @ w_gate) * (x @ w_up)) @ w_down

    x = A_q
    x = x + _A_ref(_layernorm(x, axis=-1), A_k, A_v, A_shift_k, A_ssm_k, A_ssm_D)
    x = x + _B_ref(_layernorm(x, axis=-1), B_w_gate, B_w_up, B_w_down)
    x = x + _A_ref(_layernorm(x, axis=-1), A_k, A_v, A_shift_k, A_ssm_k, A_ssm_D)
    x = x + _B_ref(_layernorm(x, axis=-1), B_w_gate, B_w_up, B_w_down)
    return x
```

```python
import numpy as np
import jax
import jax.numpy as jnp
from jax import lax
import jax.experimental.pallas as pl
import jax.experimental.pallas.tpu as pltpu

S, D, F = 2048, 448, 1792
BLK = 128
NB = S // BLK
NH = NB // 2
SH = S // 2
TM = 512
TB = TM // BLK
TH = TM // 2
NT = S // TM
FH = F // 2
DH = D // 2
KH = 256
NC = 7
RC = D // NC
R2 = 160
R2_STRIDE = 144
EPS = 1e-5
HUGE = 3.0e38
F32 = jnp.float32
BF16 = jnp.bfloat16
U32 = jnp.uint32
GELU_C0 = float(np.sqrt(2.0 / np.pi))
GELU_C1 = GELU_C0 * 0.044715
SCOPES = False


def _dft_consts():
    n = np.arange(BLK)[:, None]
    m = np.arange(BLK)[None, :]
    ang = np.pi * (((4 * m + 1) * n) % 512) / 256.0
    ft = np.concatenate([np.cos(ang), -np.sin(ang)], axis=1)
    gi = ft.T / BLK
    return jnp.asarray(ft, BF16), jnp.asarray(gi, BF16)


class _Stats:
    def __init__(self, ways=1):
        self.c = None
        self.n = 0
        self.s1 = [None] * ways
        self.s2 = [None] * ways

    def add(self, x):
        if self.c is None:
            self.c = x[0:1, :]
        xs = x - self.c
        w = self.n % len(self.s1)
        self.n += 1
        self.s1[w] = xs if self.s1[w] is None else self.s1[w] + xs
        self.s2[w] = xs * xs if self.s2[w] is None else self.s2[w] + xs * xs

    def finish(self):
        def tree(v):
            while len(v) > 1:
                v = [v[i] + v[i + 1] for i in range(0, len(v), 2)]
            return v[0]
        m = jnp.sum(tree(self.s1), axis=0, keepdims=True) * (1.0 / D)
        v = jnp.sum(tree(self.s2), axis=0, keepdims=True) * (1.0 / D) - m * m
        return self.c + m, lax.rsqrt(jnp.maximum(v, 0.0) + EPS)


def _lanes(ref, idx, start=None, size=None):
    if start is None:
        return pltpu.bitcast(ref[idx], BF16)
    return pltpu.bitcast(ref[idx, pl.ds(start, size), :], BF16)


def _put_lanes(ref, idx, val, start):
    ref[idx, pl.ds(start, val.shape[0] // 2), :] = pltpu.bitcast(val, U32)


def _a_combos(a11, a12, a21, a22):
    return [a11 + a22, a21 + a22, a11, a22, a11 + a12, a21 - a11, a12 - a22]


def _b_combos(b11, b12, b21, b22):
    return [b11 + b22, b11, b12 - b22, b21 - b11, b22, b11 + b12, b21 + b22]


def _geglu(c):
    n = c.shape[0] // 32
    g = jnp.concatenate([c[32 * i:32 * i + 16] for i in range(n)], axis=0)
    u = jnp.concatenate([c[32 * i + 16:32 * i + 32] for i in range(n)], axis=0)
    t = jnp.tanh(g * (GELU_C0 + GELU_C1 * (g * g)))
    gu = g * u
    return gu + gu * t


def _dot(a, b):
    return jnp.dot(a, b, preferred_element_type=F32)


def _tick(pace, i, n):
    if pace is None:
        return None
    r = (i * pace.shape[0] // n) // 8 * 8
    return jnp.where(pace[r:r + 8, :BLK] > HUGE, 1.0, 0.0)


def _after(x, z):
    if z is None:
        return x
    return x + jnp.tile(z, (x.shape[0] // 8, x.shape[1] // BLK))


def _token(vals):
    acc = vals[0]
    for v in vals[1:]:
        acc = acc + v
    return jnp.where(acc > HUGE, jnp.uint32(1), jnp.uint32(0))


def _gated(u, tokens):
    n = len(tokens)
    pieces, prev = [], 0
    for i, z in enumerate(tokens):
        p = ((i + 1) * u.shape[0] // n) // 8 * 8 - 8
        seg = u[p:p + 8]
        pieces += [u[prev:p]] if p > prev else []
        pieces.append(jnp.concatenate([seg[:, :BLK] | z, seg[:, BLK:]], axis=1))
        prev = p + 8
    if prev < u.shape[0]:
        pieces.append(u[prev:])
    return pltpu.bitcast(jnp.concatenate(pieces, axis=0), BF16)


class _scope:
    def __init__(self, name):
        self.cm = jax.named_scope(name) if SCOPES else None

    def __enter__(self):
        if self.cm is not None:
            self.cm.__enter__()

    def __exit__(self, *a):
        if self.cm is not None:
            self.cm.__exit__(*a)


def _kernel(q_hbm, k_hbm, v_hbm, sk_hbm, h_hbm, d_hbm, wg_hbm, wu_hbm, wd_hbm, ft_hbm, gi_hbm,
            o_hbm,
            qb, kb, vb, hb, skb, db, wgb, wub, wdb, ftb, gib,
            sg, sd, par, up, hp, hraw, y_s, x_s, st0, bs, ec, hc, ob,
            sem_small, sem_c1, sem_c2, sem_q, sem_w, sem_wd, sem_o, sem_f):
    kvh = ((k_hbm, kb), (v_hbm, vb), (h_hbm, hb))

    def fence():
        pl.semaphore_signal(sem_f, 1)
        pl.semaphore_wait(sem_f, 1)

    def c1_copy(which, g):
        src, dst = kvh[which]
        rows, cols = pl.ds(g * RC, RC), pl.ds(0, SH)
        return pltpu.make_async_copy(src.at[rows, cols], dst.at[rows, cols], sem_c1.at[which, g])

    c2_rows = ((0, 160), (160, 144), (304, 144))

    def c2_copy(which, j):
        src, dst = kvh[which]
        rows, cols = pl.ds(*c2_rows[j]), pl.ds(SH, SH)
        return pltpu.make_async_copy(src.at[rows, cols], dst.at[rows, cols], sem_c2.at[which, j])

    def w_copy(which, g):
        src, dst = ((wg_hbm, wgb), (wu_hbm, wub))[which // 2]
        cols = pl.ds((which % 2) * FH + g * BLK, BLK)
        return pltpu.make_async_copy(src.at[:, cols], dst.at[:, cols], sem_w.at[which, g])

    def q_copy(t):
        return pltpu.make_async_copy(q_hbm.at[:, pl.ds(t * TM, TM)], qb.at[t], sem_q.at[t])

    wd_copy = pltpu.make_async_copy(wd_hbm, wdb, sem_wd.at[0])

    def o_copy(t):
        return pltpu.make_async_copy(ob.at[t], o_hbm.at[:, pl.ds(t * TM, TM)], sem_o.at[t])

    small = [pltpu.make_async_copy(s, d, sem_small.at[n]) for n, (s, d) in enumerate(
        ((sk_hbm, skb), (d_hbm, db), (ft_hbm, ftb), (gi_hbm, gib)))]

    for c in small:
        c.start()
    fence()
    for g in range(NC):
        for which in range(3):
            c1_copy(which, g).start()
        fence()
    q_copy(0).start()
    fence()
    for g in range(NC):
        for which in range(4):
            w_copy(which, g).start()
        fence()
    wd_copy.start()
    fence()
    q_copy(1).start()
    fence()
    for j in range(3):
        for which in range(3):
            c2_copy(which, j).start()
        if j < 2:
            q_copy(2 + j).start()
        fence()

    for c in small:
        c.wait()
    sk = skb[...].astype(F32)
    for t in range(4):
        par[t] = jnp.broadcast_to(sk[t:t + 1, :], (BLK, D)).T
    par[4] = jnp.broadcast_to(db[...].astype(F32), (BLK, D)).T

    def conv_kv(r0, nrows, b0, pace=None):
        first = b0 == 0
        off = 0 if first else BLK
        parts = []
        for s in range(nrows // 16):
            rows = pl.ds(r0 + s * 16, 16)
            kf = _after(kb[rows, b0 * BLK - off:(b0 + NH) * BLK].astype(F32),
                        _tick(pace, s, nrows // 16))
            w = [jnp.tile(par[t, rows, :], (1, NH)) for t in range(4)]
            acc = kf[:, off:] * w[0]
            for t in range(1, 4):
                sh = pltpu.roll(kf, t, 1)[:, off:]
                if first:
                    lane = lax.broadcasted_iota(jnp.int32, (16, BLK), 1)
                    sh = jnp.concatenate([jnp.where(lane >= t, sh[:, :BLK], 0.0), sh[:, BLK:]], axis=1)
                acc = acc + sh * w[t]
            kv = (acc * vb[rows, b0 * BLK:(b0 + NH) * BLK].astype(F32)).astype(BF16)
            parts += [kv[:, a * BLK:(a + 1) * BLK] for a in range(NH)]
        return jnp.concatenate(parts, axis=0)

    def conv_fwd(r0, nrows, b0, kv):
        first = b0 == 0
        hs = hb[pl.ds(r0, nrows), b0 * BLK:(b0 + NH) * BLK]
        hst = jnp.concatenate([hs[s:s + 16, a * BLK:(a + 1) * BLK]
                               for s in range(0, nrows, 16) for a in range(NH)], axis=0)
        hf = _dot(hst, ftb[...])
        uf = _dot(kv, ftb[...])
        for gg in range(nrows // 8):
            r8 = pl.ds(r0 + gg * 8, 8)
            zp = None if first else hraw[r8, :]
            for a in range(NH):
                base = (gg // 2) * 16 * NH + a * 16 + (gg % 2) * 8
                z = uf[base:base + 8, :]
                ur, ui = z[:, :BLK], z[:, BLK:]
                for p, val in enumerate((ur + ui, ur, ui)):
                    up[p, b0 + a, r8, :] = val
                z = hf[base:base + 8, :]
                if zp is None:
                    c = z[:, :BLK] + par[4, r8, :]
                    d = z[:, BLK:]
                else:
                    c = z[:, :BLK] - zp[:, BLK:]
                    d = z[:, BLK:] + zp[:, :BLK]
                for p, val in enumerate((c, d - c, c + d)):
                    hp[p, b0 + a, r8, :] = val
                zp = z
            if first:
                hraw[r8, :] = zp

    def conv_pairs(r0, b0, tokens=None):
        b1 = b0 + NH
        ks = []
        for p in range(3):
            kp = []
            for gg in range(2):
                r8 = pl.ds(r0 + gg * 8, 8)
                uu = [up[p, a, r8, :] for a in range(b1)]
                hh = [hp[p, a, r8, :] for a in range(b1)]
                ka = []
                for a in range(b0, b1):
                    acc = hh[0] * uu[a]
                    for j in range(1, a + 1):
                        acc = acc + hh[j] * uu[a - j]
                    ka.append(acc)
                kp.append(ka)
                if tokens is not None:
                    tokens.append(_token(ka))
            ks.append([jnp.concatenate([kp[0][a], kp[1][a]], axis=0) for a in range(NH)])
        return [jnp.concatenate([(ks[0][a] - ks[2][a]).astype(BF16), (ks[0][a] + ks[1][a]).astype(BF16)],
                                axis=1) for a in range(NH)]

    def conv_inv(r0, parts, b0):
        ns = len(parts) // NH
        for tt in range(NH // TB):
            lhs = jnp.concatenate([parts[s * NH + tt * TB + a] for s in range(ns) for a in range(TB)],
                                  axis=0)
            yt = _dot(lhs, gib[...])
            cols = [jnp.concatenate([yt[(s * TB + a) * 16:(s * TB + a + 1) * 16, :] for s in range(ns)],
                                    axis=0) for a in range(TB)]
            y_s[b0 // TB + tt, pl.ds(r0, ns * 16), :] = jnp.concatenate(cols, axis=1)

    def pre_b(t, stats, pace=None):
        m, rs = stats
        st = _Stats(4)
        for r in range(0, D, 8):
            if r % 16 == 0:
                mb = _after(jnp.broadcast_to(m, (8, TM)), _tick(pace, r // 16, D // 16))
            x = x_s[t, r:r + 8, :]
            x1 = x + (x - mb) * rs * y_s[t, r:r + 8, :]
            x_s[t, r:r + 8, :] = x1
            st.add(x1)
        return st.finish()

    def pre_c(t, stats, pace=None):
        m, rs = stats
        for r in range(0, KH, 16):
            mb = _after(jnp.broadcast_to(m, (8, TM)), _tick(pace, r // 16, KH // 16))
            mb = jnp.concatenate([mb, mb], axis=0)
            hi = (x_s[t, r:r + 16, :] - mb) * rs
            if KH + r < D:
                lo = (x_s[t, KH + r:KH + r + 16, :] - mb) * rs
            else:
                lo = jnp.zeros((16, TM), F32)
            for kk, b in enumerate(_b_combos(hi[:, :TH], hi[:, TH:], lo[:, :TH], lo[:, TH:])):
                _put_lanes(bs, kk, b.astype(BF16), r // 2)

    def head(before=None, after=None):
        def prod(i, kk):
            tokens = before(i) if before is not None else None
            lhs = _gated(sg[kk], tokens) if tokens else _lanes(sg, kk)
            m = _dot(lhs, _lanes(bs, kk))
            if after is not None:
                after(i)
            return m

        m4 = prod(0, 3)
        m2 = prod(1, 1)
        m5 = prod(2, 4)
        hc[0] = _geglu(m2 + m4)
        m3 = prod(3, 2)
        m1 = prod(4, 0)
        hc[1] = _geglu(m3 + m5)
        ec[0] = (m4 - m5) + m1
        ec[1] = (m3 - m2) + m1

    def init_tile(t, tokens=None):
        st = _Stats(4)
        for r in range(0, D, 16):
            x = qb[t, r:r + 16, :].astype(F32)
            x_s[t, r:r + 16, :] = x
            st.add(x[:8])
            st.add(x[8:])
            if tokens is not None and r % 32 == 16:
                w = (st.n - 1) % 4
                tokens.append(_token([st.s2[w][:, j * BLK:(j + 1) * BLK] for j in range(TB)]))
        m, rs = st.finish()
        st0[t, 0:1, :] = m
        st0[t, 1:2, :] = rs
        return m, rs

    def tail(mid=None, mid2=None):
        m7 = _dot(_lanes(sg, 6), _lanes(bs, 6))
        h11 = _geglu(ec[0] + m7)
        m6 = _dot(_lanes(sg, 5), _lanes(bs, 5))
        h22 = _geglu(ec[1] + m6)
        if mid is not None:
            mid(m7, m6)
        h21, h12 = hc[0], hc[1]
        d2 = _dot(_lanes(sd, 1), h11.astype(BF16))
        d4 = _dot(_lanes(sd, 3), (h21 - h11).astype(BF16))
        d6 = _dot(_lanes(sd, 5), (h11 + h12).astype(BF16))
        if mid2 is not None:
            mid2()
        d5 = _dot(_lanes(sd, 4), h22.astype(BF16))
        d1 = _dot(_lanes(sd, 0), (h11 + h22).astype(BF16))
        d3 = _dot(_lanes(sd, 2), (h12 - h22).astype(BF16))
        d7 = _dot(_lanes(sd, 6), (h21 + h22).astype(BF16))
        return d1, d2, d3, d4, d5, d6, d7

    def post(t, d, final):
        d1, d2, d3, d4, d5, d6, d7 = d
        st = _Stats()
        for r in range(0, D, 16):
            if r < DH:
                q = slice(r, r + 16)
                f = jnp.concatenate([(d4[q] - d5[q]) + d1[q] + d7[q], d3[q] + d5[q]], axis=1)
            else:
                q = slice(r - DH, r - DH + 16)
                f = jnp.concatenate([d2[q] + d4[q], (d6[q] - d2[q]) + d1[q] + d3[q]], axis=1)
            xo = x_s[t, r:r + 16, :] + f
            ob[t, r:r + 16, :] = xo.astype(BF16)
            if not final:
                x_s[t, r:r + 16, :] = xo
                st.add(xo[:8])
                st.add(xo[8:])
        if not final:
            m, rs = st.finish()
            st0[t, 0:1, :] = m
            st0[t, 1:2, :] = rs

    def prep_gate_up(c):
        combos = []
        for wbuf in (wgb, wub):
            blocks = []
            for half in range(2):
                t = wbuf[:, half * FH + c * BLK: half * FH + (c + 1) * BLK].astype(F32).T
                blocks.append(t[:, :KH])
                blocks.append(jnp.concatenate([t[:, KH:], jnp.zeros((BLK, 2 * KH - D), F32)], axis=1))
            combos.append(_a_combos(*blocks))
        for kk in range(7):
            a = jnp.concatenate([combos[w][kk][16 * i:16 * i + 16]
                                 for i in range(BLK // 16) for w in range(2)], axis=0)
            _put_lanes(sg, kk, a.astype(BF16), c * BLK)

    def prep_down(lo, hi):
        tokens = []
        for r in range(lo, hi, 16):
            a11, a21 = (wdb[o + r:o + r + 16, :FH].astype(F32) * 0.5 for o in (0, DH))
            a12, a22 = (wdb[o + r:o + r + 16, FH:].astype(F32) * 0.5 for o in (0, DH))
            cs = _a_combos(a11, a12, a21, a22)
            for kk, a in enumerate(cs):
                _put_lanes(sd, kk, a.astype(BF16), r // 2)
            e = cs[0][:8] + cs[5][8:]
            tokens.append(_token([e[:, j * BLK:(j + 1) * BLK] for j in range(FH // BLK)]))
        return tokens

    def conv_first(g, carry):
        for which in range(3):
            c1_copy(which, g).wait()
        r0 = pl.multiple_of(g * RC, RC)
        conv_fwd(r0, RC, 0, conv_kv(r0, RC, 0))
        parts = []
        for s in range(RC // 16):
            parts += conv_pairs(r0 + s * 16, 0)
        conv_inv(r0, parts, 0)
        return carry

    with _scope('conv_ab'):
        lax.fori_loop(0, NC, conv_first, 0)
    with _scope('pre_a'):
        q_copy(0).wait()
        pre_c(0, pre_b(0, init_tile(0)))
    with _scope('prep'):
        for g in range(NC):
            for which in range(4):
                w_copy(which, g).wait()
            prep_gate_up(g)

    def before0(i):
        tokens = []
        if i in (0, 2):
            tokens = prep_down(i * DH // 4, (i + 2) * DH // 4)
        elif i == 4:
            init_tile(1, tokens)
        return tokens

    with _scope('head0'):
        wd_copy.wait()
        q_copy(1).wait()
        head(before0)

    def tile_of(k):
        return 2 * (k // 4) + k % 2

    groups = (3, 2, 3, 2)

    def step(k, with_conv):
        t_nxt = tile_of(k + 1)
        r0 = pl.multiple_of(k * R2_STRIDE, 16)
        box = {}

        def mid(p1, p2):
            st = (st0[t_nxt, 0:1, :], st0[t_nxt, 1:2, :])
            pre_c(t_nxt, pre_b(t_nxt, st, p1), p2)
            if with_conv:
                box['kv'] = conv_kv(r0, R2, NH, p2)

        def mid2():
            conv_fwd(r0, R2, NH, box['kv'])

        def before(i):
            tokens = []
            box['parts'] = []
            if i < len(groups):
                for s in range(groups[i]):
                    box['parts'] += conv_pairs(r0 + (sum(groups[:i]) + s) * 16, NH, tokens)
            else:
                init_tile(jnp.minimum(k + 2, NT - 1), tokens)
            return tokens

        def after(i):
            if box['parts']:
                conv_inv(r0 + sum(groups[:i]) * 16, box['parts'], NH)

        post(tile_of(k), tail(mid, mid2 if with_conv else None), False)
        if with_conv:
            head(before, after)
        else:
            head()

    def loop1(k, carry):
        for j in range(3):
            @pl.when(k == j)
            def _():
                for which in range(3):
                    c2_copy(which, j).wait()
                if j < 2:
                    q_copy(2 + j).wait()
        with _scope('step1'):
            step(k, True)
        return carry

    def loop2(k, carry):
        with _scope('step2'):
            step(k, False)
        for kk, t in ((3, 1), (6, 2)):
            @pl.when(k == kk)
            def _():
                o_copy(t).start()
        return carry

    lax.fori_loop(0, 3, loop1, 0)
    o_copy(0).start()
    lax.fori_loop(3, 7, loop2, 0)
    with _scope('epi'):
        post(NT - 1, tail(), True)
    o_copy(NT - 1).start()
    for t in range(NT):
        o_copy(t).wait()


@jax.jit
def pallas_interleave_layers__ssm_conv_h3__geglu_ffn__prompt_kernel(A_q, A_k, A_v, A_shift_k, A_ssm_k, A_ssm_D, B_x, B_w_gate, B_w_up, B_w_down):
    ft, gi = _dft_consts()
    anyspec = pl.BlockSpec(memory_space=pl.ANY)
    vm = pltpu.VMEM
    dma = pltpu.SemaphoreType.DMA
    out_t = pl.pallas_call(
        _kernel,
        in_specs=[anyspec] * 11,
        out_specs=anyspec,
        out_shape=jax.ShapeDtypeStruct((D, S), BF16),
        scratch_shapes=[
            vm((NT, D, TM), BF16), vm((D, S), BF16), vm((D, S), BF16), vm((D, S), BF16),
            vm((4, D), BF16), vm((1, D), BF16),
            vm((D, F), BF16), vm((D, F), BF16), vm((D, F), BF16),
            vm((BLK, 2 * BLK), BF16), vm((2 * BLK, BLK), BF16),
            vm((7, F // 2, KH), U32), vm((7, DH // 2, FH), U32),
            vm((5, D, BLK), F32),
            vm((3, NB, D, BLK), F32), vm((3, NB, D, BLK), F32), vm((D, 2 * BLK), F32),
            vm((NT, D, TM), F32), vm((NT, D, TM), F32), vm((NT, 8, TM), F32),
            vm((7, KH // 2, TH), U32), vm((2, F, TH), F32), vm((2, FH, TH), F32),
            vm((NT, D, TM), BF16),
            dma((4,)), dma((3, NC)), dma((3, 3)), dma((NT,)), dma((4, NC)), dma((1,)),
            dma((NT,)), pltpu.SemaphoreType.REGULAR,
        ],
        compiler_params=pltpu.CompilerParams(vmem_limit_bytes=110 * 1024 * 1024),
    )(A_q[0].T, A_k[0].T, A_v[0].T, A_shift_k.T, A_ssm_k, A_ssm_D.reshape(1, D),
      B_w_gate, B_w_up, B_w_down.T, ft, gi)
    return out_t.T[None]
```

```python
import numpy as np
import jax
import jax.numpy as jnp
from jax import lax
import jax.experimental.pallas as pl
import jax.experimental.pallas.tpu as pltpu

S, D, F = 2048, 448, 1792
BLK = 128
NB = S // BLK
NH = NB // 2
SH = S // 2
TM = 512
TB = TM // BLK
TH = TM // 2
NT = S // TM
FH = F // 2
DH = D // 2
KH = 256
NC = 7
RC = D // NC
NW1 = 4
R2 = 160
R2_STRIDE = 144
SEM_C2 = NC
SEM_W, SEM_Q0, SEM_WD, SEM_W2, SEM_OUT = (NC + 3 + i for i in range(5))
SEM_SMALL = NC + 8
SEM_W0 = NC + 9
NUM_SEMS = NC + 10
EPS = 1e-5
HUGE = 3.0e38
F32 = jnp.float32
BF16 = jnp.bfloat16
U32 = jnp.uint32
XN_SCALE = float(np.sqrt(0.5))
GELU_C0 = float(np.sqrt(2.0 / np.pi)) / XN_SCALE
GELU_C1 = float(np.sqrt(2.0 / np.pi)) * 0.044715 / XN_SCALE ** 3
SCOPES = False


def _dft_consts():
    n = np.arange(BLK)[:, None]
    m = np.arange(BLK)[None, :]
    ang = np.pi * (((4 * m + 1) * n) % 512) / 256.0
    ft = np.concatenate([np.cos(ang), -np.sin(ang)], axis=1)
    gi = ft.T / BLK
    return jnp.asarray(ft, BF16), jnp.asarray(gi, BF16)


class _Stats:
    def __init__(self, ways=1):
        self.c = None
        self.n = 0
        self.s1 = [None] * ways
        self.s2 = [None] * ways

    def add(self, x):
        if self.c is None:
            self.c = x[0:1, :]
        xs = x - self.c
        w = self.n % len(self.s1)
        self.n += 1
        self.s1[w] = xs if self.s1[w] is None else self.s1[w] + xs
        self.s2[w] = xs * xs if self.s2[w] is None else self.s2[w] + xs * xs

    def finish(self):
        def tree(v):
            while len(v) > 1:
                v = [v[i] + v[i + 1] for i in range(0, len(v), 2)]
            return v[0]
        m = jnp.sum(tree(self.s1), axis=0, keepdims=True) * (1.0 / D)
        v = jnp.sum(tree(self.s2), axis=0, keepdims=True) * (1.0 / D) - m * m
        return self.c + m, lax.rsqrt(jnp.maximum(v, 0.0) + EPS)


def _lanes(ref, idx):
    return ref[idx]


def _put_lanes(ref, idx, val, start):
    ref[idx, pl.ds(2 * start, val.shape[0]), :] = val.astype(BF16)


def _a_combos(a11, a12, a21, a22):
    return [a11 + a22, a21 + a22, a11, a22, a11 + a12, a21 - a11, a12 - a22]


def _b_combos(b11, b12, b21, b22):
    return [b11 + b22, b11, b12 - b22, b21 - b11, b22, b11 + b12, b21 + b22]


def _geglu(c):
    n = c.shape[0] // 32
    g = jnp.concatenate([c[32 * i:32 * i + 16] for i in range(n)], axis=0)
    u = jnp.concatenate([c[32 * i + 16:32 * i + 32] for i in range(n)], axis=0)
    t = jnp.tanh(g * (GELU_C0 + GELU_C1 * (g * g)))
    gu = g * u
    return gu + gu * t


def _dot(a, b):
    return jnp.dot(a, b, preferred_element_type=F32)


def _tick(pace, i, n):
    if pace is None:
        return None
    r = (i * pace.shape[0] // n) // 8 * 8
    return jnp.where(pace[r:r + 8, :BLK] > HUGE, 1.0, 0.0)


def _after(x, z):
    if z is None:
        return x
    return x + jnp.tile(z, (x.shape[0] // 8, x.shape[1] // BLK))


def _token(vals):
    acc = vals[0]
    for v in vals[1:]:
        acc = acc + v
    return jnp.where(acc > HUGE, jnp.uint32(1), jnp.uint32(0))


def _gated(u, tokens):
    n = len(tokens)
    pieces, prev = [], 0
    for i, z in enumerate(tokens):
        p = ((i + 1) * u.shape[0] // n) // 16 * 16 - 16
        seg = u[p:p + 16]
        pieces += [u[prev:p]] if p > prev else []
        first = pltpu.bitcast(pltpu.bitcast(seg[:, :BLK], U32) | z, BF16)
        pieces.append(jnp.concatenate([first, seg[:, BLK:]], axis=1) if u.shape[1] > BLK else first)
        prev = p + 16
    if prev < u.shape[0]:
        pieces.append(u[prev:])
    return jnp.concatenate(pieces, axis=0)


class _scope:
    def __init__(self, name):
        self.cm = jax.named_scope(name) if SCOPES else None

    def __enter__(self):
        if self.cm is not None:
            self.cm.__enter__()

    def __exit__(self, *a):
        if self.cm is not None:
            self.cm.__exit__(*a)


def _kernel(q_hbm, k_hbm, v_hbm, sk_hbm, h_hbm, d_hbm, wg_hbm, wu_hbm, wd_hbm, ft_hbm, gi_hbm,
            o_hbm,
            qb, kb, vb, hb, skb, db, wgb, wub, wdb, ftb, gib,
            sg, sd, par, up, hp, hraw, y_s, x_s, st0, bs, ec, hc, ob,
            sems, sem_f):
    kvh = ((k_hbm, kb), (v_hbm, vb), (h_hbm, hb))

    def fence():
        pl.semaphore_signal(sem_f, 1)
        pl.semaphore_wait(sem_f, 1)

    def c1_copy(which, g):
        src, dst = kvh[which]
        rows, cols = pl.ds(g * RC, RC), pl.ds(0, SH)
        return pltpu.make_async_copy(src.at[rows, cols], dst.at[rows, cols], sems.at[g])

    c2_rows = ((0, 160), (160, 144), (304, 144))

    def c2_copy(which, j):
        src, dst = kvh[which]
        rows, cols = pl.ds(*c2_rows[j]), pl.ds(SH, SH)
        return pltpu.make_async_copy(src.at[rows, cols], dst.at[rows, cols], sems.at[SEM_C2 + j])

    def w_copy(which, g):
        src, dst = ((wg_hbm, wgb), (wu_hbm, wub))[which // 2]
        cols = pl.ds((which % 2) * FH + g * BLK, BLK)
        return pltpu.make_async_copy(src.at[:, cols], dst.at[:, cols], sems.at[(SEM_W0, SEM_W0, SEM_W, SEM_W, SEM_W2, SEM_W2, SEM_W2)[g]])

    def q_copy(t):
        return pltpu.make_async_copy(q_hbm.at[:, pl.ds(t * TM, TM)], qb.at[t], sems.at[(SEM_Q0, SEM_WD, SEM_C2, SEM_C2 + 1)[t]])

    wd_copy = pltpu.make_async_copy(wd_hbm, wdb, sems.at[SEM_WD])

    def o_copy(t):
        return pltpu.make_async_copy(ob.at[t], o_hbm.at[:, pl.ds(t * TM, TM)], sems.at[SEM_OUT])

    small = [pltpu.make_async_copy(s, d, sems.at[SEM_SMALL]) for s, d in
             ((sk_hbm, skb), (d_hbm, db), (ft_hbm, ftb), (gi_hbm, gib))]

    for c in small:
        c.start()
    fence()
    for g in range(NC):
        for which in range(3):
            c1_copy(which, g).start()
        fence()
    q_copy(0).start()
    fence()
    for g in range(NC):
        for which in range(4):
            w_copy(which, g).start()
        fence()
    wd_copy.start()
    fence()
    q_copy(1).start()
    fence()
    for j in range(3):
        for which in range(3):
            c2_copy(which, j).start()
        if j < 2:
            q_copy(2 + j).start()
        fence()

    for c in small:
        c.wait()
    sk = skb[...].astype(F32)
    for t in range(4):
        par[t] = jnp.broadcast_to(sk[t:t + 1, :], (BLK, D)).T
    par[4] = jnp.broadcast_to(db[...].astype(F32).reshape(1, D), (BLK, D)).T

    def conv_kv(r0, nrows, b0, pace=None):
        first = b0 == 0
        off = 0 if first else BLK
        parts = []
        for s in range(nrows // 16):
            rows = pl.ds(r0 + s * 16, 16)
            kf = _after(kb[rows, b0 * BLK - off:(b0 + NH) * BLK].astype(F32),
                        _tick(pace, s, nrows // 16))
            nw = NH + off // BLK
            acc = kf[:, off:] * jnp.tile(par[0, rows, :], (1, NH))
            for t in range(1, 4):
                sh = pltpu.roll(kf * jnp.tile(par[t, rows, :], (1, nw)), t, 1)[:, off:]
                if first:
                    lane = lax.broadcasted_iota(jnp.int32, (16, BLK), 1)
                    sh = jnp.concatenate([jnp.where(lane >= t, sh[:, :BLK], 0.0), sh[:, BLK:]], axis=1)
                acc = acc + sh
            kv = acc * vb[rows, b0 * BLK:(b0 + NH) * BLK].astype(F32)
            parts += [kv[:, a * BLK:(a + 1) * BLK] for a in range(NH)]
        return jnp.concatenate(parts, axis=0).astype(BF16)

    def conv_fwd(r0, nrows, b0, kv, tokens=None):
        first = b0 == 0
        hs = hb[pl.ds(r0, nrows), b0 * BLK:(b0 + NH) * BLK]
        hst = jnp.concatenate([hs[s:s + 16, a * BLK:(a + 1) * BLK]
                               for s in range(0, nrows, 16) for a in range(NH)], axis=0)
        if tokens:
            hst = _gated(hst, tokens)
        hf = _dot(hst, ftb[...])
        uf = _dot(kv, ftb[...])
        for gg in range(nrows // 8):
            r8 = pl.ds(r0 + gg * 8, 8)
            zp = None if first else hraw[r8, :]
            for a in range(NH):
                base = (gg // 2) * 16 * NH + a * 16 + (gg % 2) * 8
                z = uf[base:base + 8, :]
                ur, ui = z[:, :BLK], z[:, BLK:]
                for p, val in enumerate((ur + ui, ur, ui)):
                    up[p, b0 + a, r8, :] = val
                z = hf[base:base + 8, :]
                if zp is None:
                    c = z[:, :BLK] + par[4, r8, :]
                    d = z[:, BLK:]
                else:
                    c = z[:, :BLK] - zp[:, BLK:]
                    d = z[:, BLK:] + zp[:, :BLK]
                for p, val in enumerate((c, d - c, c + d)):
                    hp[p, b0 + a, r8, :] = val
                zp = z
            if first:
                hraw[r8, :] = zp

    def conv_pairs(r0, b0, tokens=None):
        b1 = b0 + NH
        ks = []
        for p in range(3):
            kp = []
            for gg in range(2):
                r8 = pl.ds(r0 + gg * 8, 8)
                uu = [up[p, a, r8, :] for a in range(b1)]
                hh = [hp[p, a, r8, :] for a in range(b1)]
                ka = []
                for a in range(b0, b1):
                    acc = hh[0] * uu[a]
                    for j in range(1, a + 1):
                        acc = acc + hh[j] * uu[a - j]
                    ka.append(acc)
                kp.append(ka)
                if tokens is not None:
                    tokens.append(_token(ka))
            ks.append([jnp.concatenate([kp[0][a], kp[1][a]], axis=0) for a in range(NH)])
        return [jnp.concatenate([ks[0][a] - ks[2][a], ks[0][a] + ks[1][a]], axis=1) for a in range(NH)]

    def conv_inv(r0, parts, b0):
        ns = len(parts) // NH
        for tt in range(NH // TB):
            lhs = jnp.concatenate([parts[s * NH + tt * TB + a] for s in range(ns) for a in range(TB)],
                                  axis=0)
            yt = _dot(lhs.astype(BF16), gib[...])
            cols = [jnp.concatenate([yt[(s * TB + a) * 16:(s * TB + a + 1) * 16, :] for s in range(ns)],
                                    axis=0) for a in range(TB)]
            y_s[b0 // TB + tt, pl.ds(r0, ns * 16), :] = jnp.concatenate(cols, axis=1)

    def pre_b(t, stats, pace=None):
        m, rs = stats
        st = _Stats(4)
        for r in range(0, D, 8):
            if r % 16 == 0:
                mb = _after(jnp.broadcast_to(m, (8, TM)), _tick(pace, r // 16, D // 16))
            x = x_s[t, r:r + 8, :]
            x1 = x + (x - mb) * rs * y_s[t, r:r + 8, :]
            x_s[t, r:r + 8, :] = x1
            st.add(x1)
        return st.finish()

    def pre_c(t, stats, pace=None):
        m, rs = stats
        rs = rs * XN_SCALE
        for r in range(0, KH, 16):
            mb = _after(jnp.broadcast_to(m, (8, TM)), _tick(pace, r // 16, KH // 16))
            mb = jnp.concatenate([mb, mb], axis=0)
            hi = (x_s[t, r:r + 16, :] - mb) * rs
            if KH + r < D:
                lo = (x_s[t, KH + r:KH + r + 16, :] - mb) * rs
            else:
                lo = jnp.zeros((16, TM), F32)
            for kk, b in enumerate(_b_combos(hi[:, :TH], hi[:, TH:], lo[:, :TH], lo[:, TH:])):
                _put_lanes(bs, kk, b, r // 2)

    def head(before=None, after=None, r0=0, nr=FH):
        def prod(i, kk):
            tokens = before(i) if before is not None else None
            u = sg[kk, 2 * r0:2 * (r0 + nr), :]
            lhs = _gated(u, tokens) if tokens else u
            m = _dot(lhs, _lanes(bs, kk))
            if after is not None:
                after(i)
            return m

        m4 = prod(0, 3)
        m2 = prod(1, 1)
        hc[0, r0:r0 + nr, :] = _geglu(m2 + m4)
        m5 = prod(2, 4)
        m3 = prod(3, 2)
        hc[1, r0:r0 + nr, :] = _geglu(m3 + m5)
        m1 = prod(4, 0)
        ec[0, 2 * r0:2 * (r0 + nr), :] = (m4 - m5) + m1
        ec[1, 2 * r0:2 * (r0 + nr), :] = (m3 - m2) + m1

    init_state = {}

    def init_tile(t, tokens=None, lo=0, hi=D):
        if lo == 0:
            init_state['st'] = _Stats(4 if tokens is None else 1)
        st = init_state['st']
        for r in range(lo, hi, 16):
            x = qb[t, r:r + 16, :].astype(F32)
            x_s[t, r:r + 16, :] = x
            st.add(x[:8])
            st.add(x[8:])
            if tokens is not None and r % 32 == 16:
                e = st.s1[0] + st.s2[0]
                tokens.append(_token([e[:, j * BLK:(j + 1) * BLK] for j in range(TB)]))
        if hi < D:
            return None
        m, rs = st.finish()
        st0[t, 0:1, :] = m
        st0[t, 1:2, :] = rs
        return m, rs

    def tail(mid=None, before=None, after=None):
        def prod(i, kk, rhs):
            lhs = {2: lambda: wdb[:DH, :FH], 3: lambda: wdb[DH:, FH:]}.get(kk, lambda: sd[kk])()
            d = _dot(lhs, rhs.astype(BF16))
            if after is not None:
                after(i)
            return d

        m7 = _dot(sg[6], bs[6])
        h11 = _geglu(ec[0] + m7)
        m6 = _dot(sg[5], bs[5])
        h22 = _geglu(ec[1] + m6)
        if mid is not None:
            mid(m7, m6)
        h21, h12 = hc[0], hc[1]
        d2 = prod(0, 1, h11)
        d4 = prod(1, 3, h21 - h11)
        d6 = prod(2, 5, h11 + h12)
        d5 = prod(3, 4, h22)
        d1 = prod(4, 0, h11 + h22)
        d3 = prod(5, 2, h12 - h22)
        return d1, d2, d3, d4, d5, d6, lambda: prod(6, 6, h21 + h22)

    def post(t, d):
        d1, d2, d3, d4, d5, d6, d7 = d
        d7 = d7()
        st = _Stats()
        for r in list(range(DH, D, 16)) + list(range(0, DH, 16)):
            if r < DH:
                q = slice(r, r + 16)
                f = jnp.concatenate([(d4[q] - d5[q]) + d1[q] + d7[q], d3[q] + d5[q]], axis=1)
            else:
                q = slice(r - DH, r - DH + 16)
                f = jnp.concatenate([d2[q] + d4[q], (d6[q] - d2[q]) + d1[q] + d3[q]], axis=1)
            xo = x_s[t, r:r + 16, :] + f
            ob[t, r:r + 16, :] = xo.astype(BF16)
            x_s[t, r:r + 16, :] = xo
            st.add(xo[:8])
            st.add(xo[8:])
        m, rs = st.finish()
        st0[t, 0:1, :] = m
        st0[t, 1:2, :] = rs

    def last_copy(n):
        rows, cols = ((pl.ds(DH, DH), pl.ds(0, TM)), (pl.ds(0, DH), pl.ds(TH, TH)),
                      (pl.ds(0, DH), pl.ds(0, TH)))[n]
        dst = pl.ds((NT - 1) * TM + cols.start, cols.size)
        return pltpu.make_async_copy(ob.at[NT - 1, rows, cols], o_hbm.at[rows, dst], sems.at[SEM_OUT])

    def post_last(d):
        t = NT - 1
        d1, d2, d3, d4, d5, d6, d7 = d
        ob[t, DH:, :] = (x_s[t, DH:, :] + jnp.concatenate(
            [d2 + d4, (d6 - d2) + d1 + d3], axis=1)).astype(BF16)
        ob[t, :DH, TH:] = (x_s[t, :DH, TH:] + (d3 + d5)).astype(BF16)
        e = x_s[t, :DH, :TH] + ((d4 - d5) + d1)
        d7 = d7()
        last_copy(0).start()
        last_copy(1).start()
        ob[t, :DH, :TH] = (e + d7).astype(BF16)
        last_copy(2).start()

    def prep_gate_up(c, tokens=None):
        combos = []
        for wbuf in (wgb, wub):
            blocks = []
            for half in range(2):
                t = wbuf[:, half * FH + c * BLK: half * FH + (c + 1) * BLK].astype(F32).T
                blocks.append(t[:, :KH])
                blocks.append(jnp.concatenate([t[:, KH:], jnp.zeros((BLK, 2 * KH - D), F32)], axis=1))
            combos.append(_a_combos(*blocks))
            if tokens is not None:
                e = combos[-1][0] + combos[-1][5]
                for r in range(0, BLK, 32):
                    tokens.append(_token([e[r + i:r + i + 8, j:j + BLK]
                                          for i in range(0, 32, 8) for j in range(0, KH, BLK)]))
        for kk in range(7):
            a = jnp.concatenate([combos[w][kk][16 * i:16 * i + 16]
                                 for i in range(BLK // 16) for w in range(2)], axis=0)
            _put_lanes(sg, kk, a, c * BLK)

    def prep_down(lo, hi):
        tokens = []
        for r in range(lo, hi, 16):
            a11, a21 = (wdb[o + r:o + r + 16, :FH].astype(F32) for o in (0, DH))
            a12, a22 = (wdb[o + r:o + r + 16, FH:].astype(F32) for o in (0, DH))
            cs = _a_combos(a11, a12, a21, a22)
            for kk, a in enumerate(cs):
                if kk not in (2, 3):
                    _put_lanes(sd, kk, a, r // 2)
            e = cs[0][:8] + cs[5][8:]
            tokens.append(_token([e[:, j * BLK:(j + 1) * BLK] for j in range(FH // BLK)]))
        return tokens

    def wait_w(g):
        for which in range(4):
            w_copy(which, g).wait()

    with _scope('conv_ab'):
        parts = []
        for g in range(NC + 1):
            if g < NC:
                for which in range(3):
                    c1_copy(which, g).wait()
            if g == NC:
                q_copy(0).wait()
            if g > 1:
                conv_inv((g - 2) * RC, parts, 0)
            parts, tokens = [], []
            if g > 0:
                for s in range(RC // 16):
                    parts += conv_pairs((g - 1) * RC + s * 16, 0, tokens if g < NC else None)
            if g < NC:
                conv_fwd(g * RC, RC, 0, conv_kv(g * RC, RC, 0), tokens)
        conv_inv((NC - 1) * RC, parts, 0)
        st = pre_b(0, init_tile(0))
    with _scope('prep01'):
        wait_w(0)
        wait_w(1)
        pre_c(0, st)
        prep_gate_up(0)
        prep_gate_up(1)

    def prep_hook(chunks):
        def before(i):
            tokens = []
            if i in chunks:
                prep_gate_up(chunks[i], tokens)
            return tokens
        return before

    def before2(i):
        tokens = []
        if i == 1:
            wd_copy.wait()
            q_copy(1).wait()
        if i in (1, 2, 3, 4):
            tokens = prep_down((0, 48, 128, 176)[i - 1], (48, 128, 176, DH)[i - 1])
        if i in (2, 4):
            extra = []
            init_tile(1, extra, (i - 2) * DH // 2, i * DH // 2)
            tokens = [z for pair in zip(extra, tokens + extra) for z in pair][:2 * len(tokens)] + extra[len(tokens):]
        return tokens

    with _scope('head0a'):
        with _scope('w23'):
            wait_w(2)
            wait_w(3)
        head(prep_hook({0: 2, 2: 3}), None, 0, 2 * BLK)
    with _scope('head0b'):
        with _scope('w456'):
            for g in range(4, NC):
                wait_w(g)
        head(prep_hook({0: 4, 2: 5, 4: 6}), None, 2 * BLK, 2 * BLK)
    with _scope('head0c'):
        head(before2, None, 4 * BLK, 3 * BLK)

    def tile_of(k):
        return 2 * (k // 4) + k % 2

    groups = (4, 1, 3, 2)

    def step(k, with_conv):
        t_nxt = tile_of(k + 1)
        r0 = pl.multiple_of(k * R2_STRIDE, 16)
        box = {}

        def mid(p1, p2):
            st = (st0[t_nxt, 0:1, :], st0[t_nxt, 1:2, :])
            pre_c(t_nxt, pre_b(t_nxt, st, p1), p2)
            if with_conv:
                box['kv'] = conv_kv(r0, R2, NH, p2)

        def after_d(i):
            if i == 2:
                conv_fwd(r0, R2, NH, box['kv'])

        def before(i):
            tokens = []
            box['parts'] = []
            if i < len(groups):
                for s in range(groups[i]):
                    box['parts'] += conv_pairs(r0 + (sum(groups[:i]) + s) * 16, NH, tokens)
            else:
                init_tile(jnp.minimum(k + 2, NT - 1), tokens)
            return tokens

        def after(i):
            if box['parts']:
                conv_inv(r0 + sum(groups[:i]) * 16, box['parts'], NH)

        post(tile_of(k), tail(mid, None, after_d if with_conv else None))
        if with_conv:
            head(before, after)
        else:
            head()

    def loop1(k, carry):
        for j in range(3):
            @pl.when(k == j)
            def _():
                for which in range(3):
                    c2_copy(which, j).wait()
                if j < 2:
                    q_copy(2 + j).wait()
        with _scope('step1'):
            step(k, True)
        return carry

    def loop2(k, carry):
        with _scope('step2'):
            step(k, False)
        for kk, t in ((3, 1), (6, 2)):
            @pl.when(k == kk)
            def _():
                o_copy(t).start()
        return carry

    lax.fori_loop(0, 3, loop1, 0)
    o_copy(0).start()
    lax.fori_loop(3, 7, loop2, 0)
    with _scope('epi'):
        post_last(tail())
    for t in range(NT - 1):
        o_copy(t).wait()
    for n in range(3):
        last_copy(n).wait()


@jax.jit
def pallas_interleave_layers__ssm_conv_h3__geglu_ffn__prompt_kernel(A_q, A_k, A_v, A_shift_k, A_ssm_k, A_ssm_D, B_x, B_w_gate, B_w_up, B_w_down):
    ft, gi = _dft_consts()
    anyspec = pl.BlockSpec(memory_space=pl.ANY)
    vm = pltpu.VMEM
    dma = pltpu.SemaphoreType.DMA
    out_t = pl.pallas_call(
        _kernel,
        in_specs=[anyspec] * 11,
        out_specs=anyspec,
        out_shape=jax.ShapeDtypeStruct((D, S), BF16),
        scratch_shapes=[
            vm((NT, D, TM), BF16), vm((D, S), BF16), vm((D, S), BF16), vm((D, S), BF16),
            vm((4, D), BF16), vm((D,), BF16),
            vm((D, F), BF16), vm((D, F), BF16), vm((D, F), BF16),
            vm((BLK, 2 * BLK), BF16), vm((2 * BLK, BLK), BF16),
            vm((7, F, KH), BF16), vm((7, DH, FH), BF16),
            vm((5, D, BLK), F32),
            vm((3, NB, D, BLK), F32), vm((3, NB, D, BLK), F32), vm((D, 2 * BLK), F32),
            vm((NT, D, TM), F32), vm((NT, D, TM), F32), vm((NT, 8, TM), F32),
            vm((7, KH, TH), BF16), vm((2, F, TH), F32), vm((2, FH, TH), F32),
            vm((NT, D, TM), BF16),
            dma((NUM_SEMS,)), pltpu.SemaphoreType.REGULAR,
        ],
        compiler_params=pltpu.CompilerParams(vmem_limit_bytes=110 * 1024 * 1024),
    )(A_q[0].T, A_k[0].T, A_v[0].T, A_shift_k.T, A_ssm_k, A_ssm_D,
      B_w_gate, B_w_up, B_w_down.T, ft, gi)
    return out_t.T[None]
```

```python
import numpy as np
import jax
import jax.numpy as jnp
from jax import lax
import jax.experimental.pallas as pl
import jax.experimental.pallas.tpu as pltpu

S, D, F = 2048, 448, 1792
BLK = 128
NB = S // BLK
NH = NB // 2
SH = S // 2
TM = 512
TB = TM // BLK
TH = TM // 2
NT = S // TM
FH = F // 2
DH = D // 2
KH = 256
NC = 7
RC = D // NC
R2 = 160
R2_STRIDE = 144
C2_ROWS = ((0, 160), (160, 144), (304, 144))
PAIR_GROUPS = (4, 1, 3, 2)
N_EARLY = 8
SEM_C2 = NC
SEM_W01, SEM_W23, SEM_W46, SEM_Q0, SEM_WD, SEM_SMALL, SEM_OUT = (NC + 3 + i for i in range(7))
NUM_SEMS = NC + 10
EPS = 1e-5
HUGE = 3.0e38
F32 = jnp.float32
BF16 = jnp.bfloat16
U32 = jnp.uint32
XN_SCALE = float(np.sqrt(0.5))
GELU_C0 = float(np.sqrt(2.0 / np.pi)) / XN_SCALE
GELU_C1 = float(np.sqrt(2.0 / np.pi)) * 0.044715 / XN_SCALE ** 3


def _dft_consts():
    n = np.arange(BLK)[:, None]
    m = np.arange(BLK)[None, :]
    ang = np.pi * (((4 * m + 1) * n) % 512) / 256.0
    ft = np.concatenate([np.cos(ang), -np.sin(ang)], axis=1)
    gi = ft.T / BLK
    return jnp.asarray(ft, BF16), jnp.asarray(gi, BF16)


class _Stats:
    def __init__(self, ways=1):
        self.c = None
        self.n = 0
        self.s1 = [None] * ways
        self.s2 = [None] * ways

    def add(self, x):
        if self.c is None:
            self.c = x[0:1, :]
        xs = x - self.c
        w = self.n % len(self.s1)
        self.n += 1
        self.s1[w] = xs if self.s1[w] is None else self.s1[w] + xs
        self.s2[w] = xs * xs if self.s2[w] is None else self.s2[w] + xs * xs

    def finish(self):
        def tree(v):
            while len(v) > 1:
                v = [v[i] + v[i + 1] for i in range(0, len(v), 2)]
            return v[0]
        m = jnp.sum(tree(self.s1), axis=0, keepdims=True) * (1.0 / D)
        v = jnp.sum(tree(self.s2), axis=0, keepdims=True) * (1.0 / D) - m * m
        return self.c + m, lax.rsqrt(jnp.maximum(v, 0.0) + EPS)


def _a_combos(a11, a12, a21, a22):
    return [a11 + a22, a21 + a22, a11, a22, a11 + a12, a21 - a11, a12 - a22]


def _b_combos(b11, b12, b21, b22):
    return [b11 + b22, b11, b12 - b22, b21 - b11, b22, b11 + b12, b21 + b22]


def _geglu(c):
    n = c.shape[0] // 32
    g = jnp.concatenate([c[32 * i:32 * i + 16] for i in range(n)], axis=0)
    u = jnp.concatenate([c[32 * i + 16:32 * i + 32] for i in range(n)], axis=0)
    t = jnp.tanh(g * (GELU_C0 + GELU_C1 * (g * g)))
    gu = g * u
    return gu + gu * t


def _dot(a, b):
    return jnp.dot(a, b, preferred_element_type=F32)


def _tick(pace, i, n):
    if pace is None:
        return None
    r = (i * pace.shape[0] // n) // 8 * 8
    return jnp.where(pace[r:r + 8, :BLK] > HUGE, 1.0, 0.0)


def _after(x, z):
    if z is None:
        return x
    return x + jnp.tile(z, (x.shape[0] // 8, x.shape[1] // BLK))


def _token(vals):
    acc = vals[0]
    for v in vals[1:]:
        acc = acc + v
    return jnp.where(acc > HUGE, jnp.uint32(1), jnp.uint32(0))


def _gated(u, tokens):
    n = len(tokens)
    pieces, prev = [], 0
    for i, z in enumerate(tokens):
        p = ((i + 1) * u.shape[0] // n) // 16 * 16 - 16
        seg = u[p:p + 16]
        pieces += [u[prev:p]] if p > prev else []
        first = pltpu.bitcast(pltpu.bitcast(seg[:, :BLK], U32) | z, BF16)
        pieces.append(jnp.concatenate([first, seg[:, BLK:]], axis=1) if u.shape[1] > BLK else first)
        prev = p + 16
    if prev < u.shape[0]:
        pieces.append(u[prev:])
    return jnp.concatenate(pieces, axis=0)


def _kernel(q_hbm, k_hbm, v_hbm, sk_hbm, h_hbm, d_hbm, wg_hbm, wu_hbm, wd_hbm, ft_hbm, gi_hbm,
            o_hbm,
            qb, kb, vb, hb, skb, db, wgb, wub, wdb, ftb, gib,
            sg, sd, par, up, hp, hraw, y_s, x_s, st0, bs, ec, hc, ob,
            sems, sem_f):
    kvh = ((k_hbm, kb), (v_hbm, vb), (h_hbm, hb))

    def fence():
        pl.semaphore_signal(sem_f, 1)
        pl.semaphore_wait(sem_f, 1)

    def c1_copies(g):
        rows, cols = pl.ds(g * RC, RC), pl.ds(0, SH)
        return [pltpu.make_async_copy(src.at[rows, cols], dst.at[rows, cols], sems.at[g])
                for src, dst in kvh]

    def c2_copies(j):
        rows, cols = pl.ds(*C2_ROWS[j]), pl.ds(SH, SH)
        cs = [pltpu.make_async_copy(src.at[rows, cols], dst.at[rows, cols], sems.at[SEM_C2 + j])
              for src, dst in kvh]
        return cs + ([q_copy(2 + j)] if j < 2 else [])

    def w_copies(g):
        sem = sems.at[(SEM_W01, SEM_W01, SEM_W23, SEM_W23, SEM_W46, SEM_W46, SEM_W46)[g]]
        cs = []
        for src, dst in ((wg_hbm, wgb), (wu_hbm, wub)):
            for half in range(2):
                cols = pl.ds(half * FH + g * BLK, BLK)
                cs.append(pltpu.make_async_copy(src.at[:, cols], dst.at[:, cols], sem))
        return cs

    def q_copy(t):
        sem = sems.at[(SEM_Q0, SEM_WD, SEM_C2, SEM_C2 + 1)[t]]
        return pltpu.make_async_copy(q_hbm.at[:, pl.ds(t * TM, TM)], qb.at[t], sem)

    wd_copy = pltpu.make_async_copy(wd_hbm, wdb, sems.at[SEM_WD])

    def o_copy(t):
        return pltpu.make_async_copy(ob.at[t], o_hbm.at[:, pl.ds(t * TM, TM)], sems.at[SEM_OUT])

    def last_copy(n):
        rows, cols = ((pl.ds(DH, DH), pl.ds(0, TM)), (pl.ds(0, DH), pl.ds(TH, TH)),
                      (pl.ds(0, DH), pl.ds(0, TH)))[n]
        dst = pl.ds((NT - 1) * TM + cols.start, cols.size)
        return pltpu.make_async_copy(ob.at[NT - 1, rows, cols], o_hbm.at[rows, dst],
                                     sems.at[SEM_OUT])

    small = [pltpu.make_async_copy(s, d, sems.at[SEM_SMALL]) for s, d in
             ((sk_hbm, skb), (d_hbm, db), (ft_hbm, ftb), (gi_hbm, gib))]

    def wait(copies):
        for c in copies:
            c.wait()

    for group in ([small] + [c1_copies(g) for g in range(NC)] + [[q_copy(0)]]
                  + [w_copies(g) for g in range(NC)] + [[wd_copy], [q_copy(1)]]
                  + [c2_copies(j) for j in range(3)]):
        for c in group:
            c.start()
        fence()

    wait(small)
    sk = skb[...].astype(F32)
    for t in range(4):
        par[t] = jnp.broadcast_to(sk[t:t + 1, :], (BLK, D)).T
    par[4] = jnp.broadcast_to(db[...].astype(F32).reshape(1, D), (BLK, D)).T

    def conv_kv(r0, nrows, b0, pace=None):
        first = b0 == 0
        off = 0 if first else BLK
        parts = []
        for s in range(nrows // 16):
            rows = pl.ds(r0 + s * 16, 16)
            kf = _after(kb[rows, b0 * BLK - off:(b0 + NH) * BLK].astype(F32),
                        _tick(pace, s, nrows // 16))
            nw = NH + off // BLK
            acc = kf[:, off:] * jnp.tile(par[0, rows, :], (1, NH))
            for t in range(1, 4):
                sh = pltpu.roll(kf * jnp.tile(par[t, rows, :], (1, nw)), t, 1)[:, off:]
                if first:
                    lane = lax.broadcasted_iota(jnp.int32, (16, BLK), 1)
                    sh = jnp.concatenate([jnp.where(lane >= t, sh[:, :BLK], 0.0), sh[:, BLK:]],
                                         axis=1)
                acc = acc + sh
            kv = acc * vb[rows, b0 * BLK:(b0 + NH) * BLK].astype(F32)
            parts += [kv[:, a * BLK:(a + 1) * BLK] for a in range(NH)]
        return jnp.concatenate(parts, axis=0).astype(BF16)

    def conv_fwd(r0, nrows, b0, kv, tokens=None):
        first = b0 == 0
        hs = hb[pl.ds(r0, nrows), b0 * BLK:(b0 + NH) * BLK]
        hst = jnp.concatenate([hs[s:s + 16, a * BLK:(a + 1) * BLK]
                               for s in range(0, nrows, 16) for a in range(NH)], axis=0)
        if tokens:
            hst = _gated(hst, tokens)
        hf = _dot(hst, ftb[...])
        uf = _dot(kv, ftb[...])
        for gg in range(nrows // 8):
            r8 = pl.ds(r0 + gg * 8, 8)
            zp = None if first else hraw[r8, :]
            for a in range(NH):
                base = (gg // 2) * 16 * NH + a * 16 + (gg % 2) * 8
                z = uf[base:base + 8, :]
                ur, ui = z[:, :BLK], z[:, BLK:]
                for p, val in enumerate((ur + ui, ur, ui)):
                    up[p, b0 + a, r8, :] = val
                z = hf[base:base + 8, :]
                if zp is None:
                    c = z[:, :BLK] + par[4, r8, :]
                    d = z[:, BLK:]
                else:
                    c = z[:, :BLK] - zp[:, BLK:]
                    d = z[:, BLK:] + zp[:, :BLK]
                for p, val in enumerate((c, d - c, c + d)):
                    hp[p, b0 + a, r8, :] = val
                zp = z
            if first:
                hraw[r8, :] = zp

    def conv_pairs(r0, b0, tokens=None):
        b1 = b0 + NH
        ks = []
        for p in range(3):
            kp = []
            for gg in range(2):
                r8 = pl.ds(r0 + gg * 8, 8)
                uu = [up[p, a, r8, :] for a in range(b1)]
                hh = [hp[p, a, r8, :] for a in range(b1)]
                ka = []
                for a in range(b0, b1):
                    acc = hh[0] * uu[a]
                    for j in range(1, a + 1):
                        acc = acc + hh[j] * uu[a - j]
                    ka.append(acc)
                kp.append(ka)
                if tokens is not None:
                    tokens.append(_token(ka))
            ks.append([jnp.concatenate([kp[0][a], kp[1][a]], axis=0) for a in range(NH)])
        return [jnp.concatenate([ks[0][a] - ks[2][a], ks[0][a] + ks[1][a]], axis=1)
                for a in range(NH)]

    def conv_inv(r0, parts, b0):
        ns = len(parts) // NH
        for tt in range(NH // TB):
            lhs = jnp.concatenate(
                [parts[s * NH + tt * TB + a] for s in range(ns) for a in range(TB)], axis=0)
            yt = _dot(lhs.astype(BF16), gib[...])
            cols = [jnp.concatenate(
                [yt[(s * TB + a) * 16:(s * TB + a + 1) * 16, :] for s in range(ns)], axis=0)
                for a in range(TB)]
            y_s[b0 // TB + tt, pl.ds(r0, ns * 16), :] = jnp.concatenate(cols, axis=1)

    def gate_layer(t, stats, pace=None):
        m, rs = stats
        st = _Stats(4)
        for r in range(0, D, 8):
            if r % 16 == 0:
                mb = _after(jnp.broadcast_to(m, (8, TM)), _tick(pace, r // 16, D // 16))
            x = x_s[t, r:r + 8, :]
            x1 = x + (x - mb) * rs * y_s[t, r:r + 8, :]
            x_s[t, r:r + 8, :] = x1
            st.add(x1)
        return st.finish()

    def ffn_operands(t, stats, pace=None):
        m, rs = stats
        rs = rs * XN_SCALE
        for r in range(0, KH, 16):
            mb = _after(jnp.broadcast_to(m, (8, TM)), _tick(pace, r // 16, KH // 16))
            mb = jnp.concatenate([mb, mb], axis=0)
            hi = (x_s[t, r:r + 16, :] - mb) * rs
            if KH + r < D:
                lo = (x_s[t, KH + r:KH + r + 16, :] - mb) * rs
            else:
                lo = jnp.zeros((16, TM), F32)
            for kk, b in enumerate(_b_combos(hi[:, :TH], hi[:, TH:], lo[:, :TH], lo[:, TH:])):
                bs[kk, r:r + 16, :] = b.astype(BF16)

    def head(before=None, after=None, r0=0, nr=FH):
        def prod(i, kk):
            tokens = before(i) if before is not None else None
            u = sg[kk, 2 * r0:2 * (r0 + nr), :]
            lhs = _gated(u, tokens) if tokens else u
            m = _dot(lhs, bs[kk])
            if after is not None:
                after(i)
            return m

        m4 = prod(0, 3)
        m2 = prod(1, 1)
        hc[0, r0:r0 + nr, :] = _geglu(m2 + m4)
        m5 = prod(2, 4)
        m3 = prod(3, 2)
        hc[1, r0:r0 + nr, :] = _geglu(m3 + m5)
        m1 = prod(4, 0)
        ec[0, 2 * r0:2 * (r0 + nr), :] = (m4 - m5) + m1
        ec[1, 2 * r0:2 * (r0 + nr), :] = (m3 - m2) + m1

    init_state = {}

    def init_tile(t, tokens=None, lo=0, hi=D):
        if lo == 0:
            init_state['st'] = _Stats(4 if tokens is None else 1)
        st = init_state['st']
        for r in range(lo, hi, 16):
            x = qb[t, r:r + 16, :].astype(F32)
            x_s[t, r:r + 16, :] = x
            st.add(x[:8])
            st.add(x[8:])
            if tokens is not None and r % 32 == 16:
                e = st.s1[0] + st.s2[0]
                tokens.append(_token([e[:, j * BLK:(j + 1) * BLK] for j in range(TB)]))
        if hi < D:
            return None
        m, rs = st.finish()
        st0[t, 0:1, :] = m
        st0[t, 1:2, :] = rs
        return m, rs

    def tail(mid=None, after=None):
        def prod(i, kk, rhs):
            lhs = wdb[:DH, :FH] if kk == 2 else wdb[DH:, FH:] if kk == 3 else sd[kk]
            d = _dot(lhs, rhs.astype(BF16))
            if after is not None:
                after(i)
            return d

        m7 = _dot(sg[6], bs[6])
        h11 = _geglu(ec[0] + m7)
        m6 = _dot(sg[5], bs[5])
        h22 = _geglu(ec[1] + m6)
        if mid is not None:
            mid(m7, m6)
        h21, h12 = hc[0], hc[1]
        d2 = prod(0, 1, h11)
        d4 = prod(1, 3, h21 - h11)
        d6 = prod(2, 5, h11 + h12)
        d5 = prod(3, 4, h22)
        d1 = prod(4, 0, h11 + h22)
        d3 = prod(5, 2, h12 - h22)
        return d1, d2, d3, d4, d5, d6, lambda: prod(6, 6, h21 + h22)

    def residual(t, d):
        d1, d2, d3, d4, d5, d6, d7 = d
        d7 = d7()
        st = _Stats()
        for r in list(range(DH, D, 16)) + list(range(0, DH, 16)):
            if r < DH:
                q = slice(r, r + 16)
                f = jnp.concatenate([(d4[q] - d5[q]) + d1[q] + d7[q], d3[q] + d5[q]], axis=1)
            else:
                q = slice(r - DH, r - DH + 16)
                f = jnp.concatenate([d2[q] + d4[q], (d6[q] - d2[q]) + d1[q] + d3[q]], axis=1)
            xo = x_s[t, r:r + 16, :] + f
            ob[t, r:r + 16, :] = xo.astype(BF16)
            x_s[t, r:r + 16, :] = xo
            st.add(xo[:8])
            st.add(xo[8:])
        m, rs = st.finish()
        st0[t, 0:1, :] = m
        st0[t, 1:2, :] = rs

    def residual_last(d):
        t = NT - 1
        d1, d2, d3, d4, d5, d6, d7 = d
        ob[t, DH:, :] = (x_s[t, DH:, :] + jnp.concatenate(
            [d2 + d4, (d6 - d2) + d1 + d3], axis=1)).astype(BF16)
        ob[t, :DH, TH:] = (x_s[t, :DH, TH:] + (d3 + d5)).astype(BF16)
        e = x_s[t, :DH, :TH] + ((d4 - d5) + d1)
        d7 = d7()
        last_copy(0).start()
        last_copy(1).start()
        ob[t, :DH, :TH] = (e + d7).astype(BF16)
        last_copy(2).start()

    def prep_gate_up(c, tokens=None):
        combos = []
        for wbuf in (wgb, wub):
            blocks = []
            for half in range(2):
                t = wbuf[:, half * FH + c * BLK: half * FH + (c + 1) * BLK].astype(F32).T
                blocks.append(t[:, :KH])
                blocks.append(jnp.concatenate([t[:, KH:], jnp.zeros((BLK, 2 * KH - D), F32)],
                                              axis=1))
            combos.append(_a_combos(*blocks))
            if tokens is not None:
                e = combos[-1][0] + combos[-1][5]
                for r in range(0, BLK, 32):
                    tokens.append(_token([e[r + i:r + i + 8, j:j + BLK]
                                          for i in range(0, 32, 8) for j in range(0, KH, BLK)]))
        for kk in range(7):
            a = jnp.concatenate([combos[w][kk][16 * i:16 * i + 16]
                                 for i in range(BLK // 16) for w in range(2)], axis=0)
            sg[kk, 2 * c * BLK:2 * (c + 1) * BLK, :] = a.astype(BF16)

    def prep_down(lo, hi):
        tokens = []
        for r in range(lo, hi, 16):
            a11, a21 = (wdb[o + r:o + r + 16, :FH].astype(F32) for o in (0, DH))
            a12, a22 = (wdb[o + r:o + r + 16, FH:].astype(F32) for o in (0, DH))
            cs = _a_combos(a11, a12, a21, a22)
            for kk, a in enumerate(cs):
                if kk not in (2, 3):
                    sd[kk, r:r + 16, :] = a.astype(BF16)
            e = cs[0][:8] + cs[5][8:]
            tokens.append(_token([e[:, j * BLK:(j + 1) * BLK] for j in range(FH // BLK)]))
        return tokens

    parts = []
    for g in range(NC + 1):
        wait(c1_copies(g) if g < NC else [q_copy(0)])
        done, parts, tokens = parts, [], []
        if g > 0:
            for s in range(RC // 16):
                parts += conv_pairs((g - 1) * RC + s * 16, 0, tokens if g < NC else None)
        if g > 1:
            early, tokens = tokens[:N_EARLY], tokens[N_EARLY:]
            for n, z in enumerate(early):
                i = ((n // 2 + 1) * (RC // 16) // (N_EARLY // 2) - 1) * NH + (n % 2) * TB + TB - 1
                p = done[i]
                top = jnp.concatenate(
                    [p[:8, :BLK] + z.astype(jnp.int32).astype(F32), p[:8, BLK:]], axis=1)
                done[i] = jnp.concatenate([top, p[8:]], axis=0)
            conv_inv((g - 2) * RC, done, 0)
        if g < NC:
            conv_fwd(g * RC, RC, 0, conv_kv(g * RC, RC, 0), tokens)
    conv_inv((NC - 1) * RC, parts, 0)
    st = gate_layer(0, init_tile(0))
    wait(w_copies(0) + w_copies(1))
    ffn_operands(0, st)
    prep_gate_up(0)
    prep_gate_up(1)

    def prep_hook(chunks, wait_at):
        def before(i):
            tokens = []
            if i == wait_at:
                wait([c for g in chunks.values() for c in w_copies(g)])
            if i in chunks:
                prep_gate_up(chunks[i], tokens)
            return tokens
        return before

    def down_hook(i):
        tokens = []
        if i == 1:
            wait([wd_copy, q_copy(1)])
        if i > 0:
            tokens = prep_down((0, 48, 128, 176)[i - 1], (48, 128, 176, DH)[i - 1])
        if i in (2, 4):
            extra = []
            init_tile(1, extra, (i - 2) * DH // 2, i * DH // 2)
            tokens = [z for pair in zip(extra, tokens) for z in pair] + extra[len(tokens):]
        return tokens

    head(prep_hook({2: 2, 4: 3}, 2), None, 0, 2 * BLK)
    head(prep_hook({0: 4, 2: 5, 4: 6}, 0), None, 2 * BLK, 2 * BLK)
    head(down_hook, None, 4 * BLK, 3 * BLK)

    def tile_of(k):
        return 2 * (k // 4) + k % 2

    def step(k, with_conv):
        t_nxt = tile_of(k + 1)
        r0 = pl.multiple_of(k * R2_STRIDE, 16)
        box = {}

        def mid(m7, m6):
            st = (st0[t_nxt, 0:1, :], st0[t_nxt, 1:2, :])
            ffn_operands(t_nxt, gate_layer(t_nxt, st, m7), m6)
            if with_conv:
                box['kv'] = conv_kv(r0, R2, NH, m6)

        def after_down(i):
            if i == 2:
                conv_fwd(r0, R2, NH, box['kv'])

        def before(i):
            tokens = []
            box['parts'] = []
            if i < len(PAIR_GROUPS):
                for s in range(PAIR_GROUPS[i]):
                    box['parts'] += conv_pairs(r0 + (sum(PAIR_GROUPS[:i]) + s) * 16, NH, tokens)
            else:
                init_tile(jnp.minimum(k + 2, NT - 1), tokens)
            return tokens

        def after(i):
            if box['parts']:
                conv_inv(r0 + sum(PAIR_GROUPS[:i]) * 16, box['parts'], NH)

        residual(tile_of(k), tail(mid, after_down if with_conv else None))
        if with_conv:
            head(before, after)
        else:
            head()

    def loop1(k, carry):
        for j in range(3):
            @pl.when(k == j)
            def _():
                wait(c2_copies(j))
        step(k, True)
        return carry

    def loop2(k, carry):
        step(k, False)
        for kk, t in ((3, 1), (6, 2)):
            @pl.when(k == kk)
            def _():
                o_copy(t).start()
        return carry

    lax.fori_loop(0, 3, loop1, 0)
    o_copy(0).start()
    lax.fori_loop(3, 7, loop2, 0)
    residual_last(tail())
    wait([o_copy(t) for t in range(NT - 1)] + [last_copy(n) for n in range(3)])


@jax.jit
def pallas_interleave_layers__ssm_conv_h3__geglu_ffn__prompt_kernel(A_q, A_k, A_v, A_shift_k, A_ssm_k, A_ssm_D, B_x, B_w_gate, B_w_up, B_w_down):
    ft, gi = _dft_consts()
    anyspec = pl.BlockSpec(memory_space=pl.ANY)
    vm = pltpu.VMEM
    out_t = pl.pallas_call(
        _kernel,
        in_specs=[anyspec] * 11,
        out_specs=anyspec,
        out_shape=jax.ShapeDtypeStruct((D, S), BF16),
        scratch_shapes=[
            vm((NT, D, TM), BF16), vm((D, S), BF16), vm((D, S), BF16), vm((D, S), BF16),
            vm((4, D), BF16), vm((D,), BF16),
            vm((D, F), BF16), vm((D, F), BF16), vm((D, F), BF16),
            vm((BLK, 2 * BLK), BF16), vm((2 * BLK, BLK), BF16),
            vm((7, F, KH), BF16), vm((7, DH, FH), BF16),
            vm((5, D, BLK), F32),
            vm((3, NB, D, BLK), F32), vm((3, NB, D, BLK), F32), vm((D, 2 * BLK), F32),
            vm((NT, D, TM), F32), vm((NT, D, TM), F32), vm((NT, 8, TM), F32),
            vm((7, KH, TH), BF16), vm((2, F, TH), F32), vm((2, FH, TH), F32),
            vm((NT, D, TM), BF16),
            pltpu.SemaphoreType.DMA((NUM_SEMS,)), pltpu.SemaphoreType.REGULAR,
        ],
        compiler_params=pltpu.CompilerParams(vmem_limit_bytes=110 * 1024 * 1024),
    )(A_q[0].T, A_k[0].T, A_v[0].T, A_shift_k.T, A_ssm_k, A_ssm_D,
      B_w_gate, B_w_up, B_w_down.T, ft, gi)
    return out_t.T[None]
```

```python
import numpy as np
import jax
import jax.numpy as jnp
from jax import lax
import jax.experimental.pallas as pl
import jax.experimental.pallas.tpu as pltpu

S, D, F = 2048, 448, 1792
BLK = 128
NB = S // BLK
NH = NB // 2
SH = S // 2
TM = 512
TB = TM // BLK
TH = TM // 2
NT = S // TM
FH = F // 2
DH = D // 2
KH = 256
NC = 7
RC = D // NC
R2 = 160
R2_STRIDE = 144
C2_ROWS = ((0, 160), (160, 144), (304, 144))
PAIR_GROUPS = (4, 1, 3, 2)
N_EARLY = 8
SEM_C2 = NC
SEM_W01, SEM_W23, SEM_W46, SEM_Q0, SEM_WD, SEM_SMALL, SEM_OUT = (NC + 3 + i for i in range(7))
NUM_SEMS = NC + 10
EPS = 1e-5
HUGE = 3.0e38
F32 = jnp.float32
BF16 = jnp.bfloat16
U32 = jnp.uint32
XN_SCALE = float(np.sqrt(0.5))
GELU_C0 = float(np.sqrt(2.0 / np.pi)) / XN_SCALE
GELU_C1 = float(np.sqrt(2.0 / np.pi)) * 0.044715 / XN_SCALE ** 3


def _dft_consts():
    n = np.arange(BLK)[:, None]
    m = np.arange(BLK)[None, :]
    ang = np.pi * (((4 * m + 1) * n) % 512) / 256.0
    ft = np.concatenate([np.cos(ang), -np.sin(ang)], axis=1)
    gi = ft.T / BLK
    return jnp.asarray(ft, BF16), jnp.asarray(gi, BF16)


class _Stats:
    def __init__(self, ways=1):
        self.c = None
        self.n = 0
        self.s1 = [None] * ways
        self.s2 = [None] * ways

    def add(self, x):
        if self.c is None:
            self.c = x[0:1, :]
        xs = x - self.c
        w = self.n % len(self.s1)
        self.n += 1
        self.s1[w] = xs if self.s1[w] is None else self.s1[w] + xs
        self.s2[w] = xs * xs if self.s2[w] is None else self.s2[w] + xs * xs

    def finish(self):
        def tree(v):
            while len(v) > 1:
                v = [v[i] + v[i + 1] for i in range(0, len(v), 2)]
            return v[0]
        m = jnp.sum(tree(self.s1), axis=0, keepdims=True) * (1.0 / D)
        v = jnp.sum(tree(self.s2), axis=0, keepdims=True) * (1.0 / D) - m * m
        return self.c + m, lax.rsqrt(jnp.maximum(v, 0.0) + EPS)


def _a_combos(a11, a12, a21, a22):
    return [a11 + a22, a21 + a22, a11, a22, a11 + a12, a21 - a11, a12 - a22]


def _b_combos(b11, b12, b21, b22):
    return [b11 + b22, b11, b12 - b22, b21 - b11, b22, b11 + b12, b21 + b22]


def _geglu(c):
    n = c.shape[0] // 32
    g = jnp.concatenate([c[32 * i:32 * i + 16] for i in range(n)], axis=0)
    u = jnp.concatenate([c[32 * i + 16:32 * i + 32] for i in range(n)], axis=0)
    t = jnp.tanh(g * (GELU_C0 + GELU_C1 * (g * g)))
    gu = g * u
    return gu + gu * t


def _dot(a, b):
    return jnp.dot(a, b, preferred_element_type=F32)


def _tick(pace, i, n):
    if pace is None:
        return None
    r = (i * pace.shape[0] // n) // 8 * 8
    return jnp.where(pace[r:r + 8, :BLK] > HUGE, 1.0, 0.0)


def _after(x, z):
    if z is None:
        return x
    return x + jnp.tile(z, (x.shape[0] // 8, x.shape[1] // BLK))


def _token(vals):
    acc = vals[0]
    for v in vals[1:]:
        acc = acc + v
    return jnp.where(acc > HUGE, jnp.uint32(1), jnp.uint32(0))


def _gated(u, tokens):
    n = len(tokens)
    pieces, prev = [], 0
    for i, z in enumerate(tokens):
        p = ((i + 1) * u.shape[0] // n) // 16 * 16 - 16
        seg = u[p:p + 16]
        pieces += [u[prev:p]] if p > prev else []
        first = pltpu.bitcast(pltpu.bitcast(seg[:, :BLK], U32) | z, BF16)
        pieces.append(jnp.concatenate([first, seg[:, BLK:]], axis=1) if u.shape[1] > BLK else first)
        prev = p + 16
    if prev < u.shape[0]:
        pieces.append(u[prev:])
    return jnp.concatenate(pieces, axis=0)


def _kernel(q_hbm, k_hbm, v_hbm, sk_hbm, h_hbm, d_hbm, wg_hbm, wu_hbm, wd_hbm, ft_hbm, gi_hbm,
            o_hbm,
            qb, kb, vb, hb, skb, db, wgb, wub, wdb, ftb, gib,
            sg, sd, par, up, hp, hraw, y_s, x_s, st0, bs, ec, hc, ob,
            sems, sem_f):
    kvh = ((k_hbm, kb), (v_hbm, vb), (h_hbm, hb))

    def fence():
        pl.semaphore_signal(sem_f, 1)
        pl.semaphore_wait(sem_f, 1)

    def c1_copies(g):
        rows, cols = pl.ds(g * RC, RC), pl.ds(0, SH)
        return [pltpu.make_async_copy(src.at[rows, cols], dst.at[rows, cols], sems.at[g])
                for src, dst in kvh]

    def c2_copies(j):
        rows, cols = pl.ds(*C2_ROWS[j]), pl.ds(SH, SH)
        cs = [pltpu.make_async_copy(src.at[rows, cols], dst.at[rows, cols], sems.at[SEM_C2 + j])
              for src, dst in kvh]
        return cs + ([q_copy(2 + j)] if j < 2 else [])

    def w_copies(g):
        sem = sems.at[(SEM_W01, SEM_W01, SEM_W23, SEM_W23, SEM_W46, SEM_W46, SEM_W46)[g]]
        cs = []
        for src, dst in ((wg_hbm, wgb), (wu_hbm, wub)):
            for half in range(2):
                cols = pl.ds(half * FH + g * BLK, BLK)
                cs.append(pltpu.make_async_copy(src.at[:, cols], dst.at[:, cols], sem))
        return cs

    def q_copy(t):
        sem = sems.at[(SEM_Q0, SEM_WD, SEM_C2, SEM_C2 + 1)[t]]
        return pltpu.make_async_copy(q_hbm.at[:, pl.ds(t * TM, TM)], qb.at[t], sem)

    wd_copy = pltpu.make_async_copy(wd_hbm, wdb, sems.at[SEM_WD])

    def o_copy(t):
        return pltpu.make_async_copy(ob.at[t], o_hbm.at[:, pl.ds(t * TM, TM)], sems.at[SEM_OUT])

    def last_copy(n):
        rows, cols = ((pl.ds(DH, DH), pl.ds(0, TM)), (pl.ds(0, DH), pl.ds(TH, TH)),
                      (pl.ds(0, DH), pl.ds(0, TH)))[n]
        dst = pl.ds((NT - 1) * TM + cols.start, cols.size)
        return pltpu.make_async_copy(ob.at[NT - 1, rows, cols], o_hbm.at[rows, dst],
                                     sems.at[SEM_OUT])

    small = [pltpu.make_async_copy(s, d, sems.at[SEM_SMALL]) for s, d in
             ((sk_hbm, skb), (d_hbm, db), (ft_hbm, ftb), (gi_hbm, gib))]

    def wait(copies):
        for c in copies:
            c.wait()

    for group in ([small] + [c1_copies(g) for g in range(NC)] + [[q_copy(0)]]
                  + [w_copies(g) for g in range(NC)] + [[wd_copy], [q_copy(1)]]
                  + [c2_copies(j) for j in range(3)]):
        for c in group:
            c.start()
        fence()

    wait(small)
    sk = skb[...].astype(F32)
    for t in range(4):
        par[t] = jnp.broadcast_to(sk[t:t + 1, :], (BLK, D)).T
    par[4] = jnp.broadcast_to(db[...].astype(F32).reshape(1, D), (BLK, D)).T

    def conv_kv(r0, nrows, b0, pace=None):
        first = b0 == 0
        off = 0 if first else BLK
        parts = []
        for s in range(nrows // 16):
            rows = pl.ds(r0 + s * 16, 16)
            kf = _after(kb[rows, b0 * BLK - off:(b0 + NH) * BLK].astype(F32),
                        _tick(pace, s, nrows // 16))
            nw = NH + off // BLK
            acc = kf[:, off:] * jnp.tile(par[0, rows, :], (1, NH))
            for t in range(1, 4):
                sh = pltpu.roll(kf * jnp.tile(par[t, rows, :], (1, nw)), t, 1)[:, off:]
                if first:
                    lane = lax.broadcasted_iota(jnp.int32, (16, BLK), 1)
                    sh = jnp.concatenate([jnp.where(lane >= t, sh[:, :BLK], 0.0), sh[:, BLK:]],
                                         axis=1)
                acc = acc + sh
            kv = acc * vb[rows, b0 * BLK:(b0 + NH) * BLK].astype(F32)
            parts += [kv[:, a * BLK:(a + 1) * BLK] for a in range(NH)]
        return jnp.concatenate(parts, axis=0).astype(BF16)

    def conv_fwd(r0, nrows, b0, kv, tokens=None):
        first = b0 == 0
        hs = hb[pl.ds(r0, nrows), b0 * BLK:(b0 + NH) * BLK]
        hst = jnp.concatenate([hs[s:s + 16, a * BLK:(a + 1) * BLK]
                               for s in range(0, nrows, 16) for a in range(NH)], axis=0)
        if tokens:
            hst = _gated(hst, tokens)
        hf = _dot(hst, ftb[...])
        uf = _dot(kv, ftb[...])
        for gg in range(nrows // 8):
            r8 = pl.ds(r0 + gg * 8, 8)
            zp = None if first else hraw[r8, :]
            us, hs = [], []
            for a in range(NH):
                base = (gg // 2) * 16 * NH + a * 16 + (gg % 2) * 8
                z = uf[base:base + 8, :]
                ur, ui = z[:, :BLK], z[:, BLK:]
                us.append((ur + ui, ur, ui))
                z = hf[base:base + 8, :]
                if zp is None:
                    c = z[:, :BLK] + par[4, r8, :]
                    d = z[:, BLK:]
                else:
                    c = z[:, :BLK] - zp[:, BLK:]
                    d = z[:, BLK:] + zp[:, :BLK]
                hs.append((c, d - c, c + d))
                zp = z
            for p in range(3):
                up[p, b0:b0 + NH, r8, :] = jnp.stack([t[p] for t in us])
                hp[p, b0:b0 + NH, r8, :] = jnp.stack([t[p] for t in hs])
            if first:
                hraw[r8, :] = zp

    def conv_pairs(r0, b0, tokens=None):
        b1 = b0 + NH
        ks = []
        for p in range(3):
            kp = []
            for gg in range(2):
                r8 = pl.ds(r0 + gg * 8, 8)
                uu = up[p, :b1, r8, :]
                hh = hp[p, :b1, r8, :]
                ka = []
                for a in range(b0, b1):
                    acc = hh[0] * uu[a]
                    for j in range(1, a + 1):
                        acc = acc + hh[j] * uu[a - j]
                    ka.append(acc)
                kp.append(ka)
                if tokens is not None:
                    tokens.append(_token(ka))
            ks.append([jnp.concatenate([kp[0][a], kp[1][a]], axis=0) for a in range(NH)])
        return [jnp.concatenate([ks[0][a] - ks[2][a], ks[0][a] + ks[1][a]], axis=1)
                for a in range(NH)]

    def conv_inv(r0, parts, b0):
        ns = len(parts) // NH
        for tt in range(NH // TB):
            lhs = jnp.concatenate(
                [parts[s * NH + tt * TB + a] for s in range(ns) for a in range(TB)], axis=0)
            yt = _dot(lhs.astype(BF16), gib[...])
            cols = [jnp.concatenate(
                [yt[(s * TB + a) * 16:(s * TB + a + 1) * 16, :] for s in range(ns)], axis=0)
                for a in range(TB)]
            y_s[b0 // TB + tt, pl.ds(r0, ns * 16), :] = jnp.concatenate(cols, axis=1)

    def gate_layer(t, stats, pace=None):
        m, rs = stats
        st = _Stats(4)
        for r in range(0, D, 8):
            if r % 16 == 0:
                mb = _after(jnp.broadcast_to(m, (8, TM)), _tick(pace, r // 16, D // 16))
            x = x_s[t, r:r + 8, :]
            x1 = x + (x - mb) * rs * y_s[t, r:r + 8, :]
            x_s[t, r:r + 8, :] = x1
            st.add(x1)
        return st.finish()

    def ffn_operands(t, stats, pace=None):
        m, rs = stats
        rs = rs * XN_SCALE
        for r in range(0, KH, 16):
            mb = _after(jnp.broadcast_to(m, (8, TM)), _tick(pace, r // 16, KH // 16))
            mb = jnp.concatenate([mb, mb], axis=0)
            hi = (x_s[t, r:r + 16, :] - mb) * rs
            if KH + r < D:
                lo = (x_s[t, KH + r:KH + r + 16, :] - mb) * rs
            else:
                lo = jnp.zeros((16, TM), F32)
            for kk, b in enumerate(_b_combos(hi[:, :TH], hi[:, TH:], lo[:, :TH], lo[:, TH:])):
                bs[kk, r:r + 16, :] = b.astype(BF16)

    def head(before=None, after=None, r0=0, nr=FH):
        def prod(i, kk):
            tokens = before(i) if before is not None else None
            u = sg[kk, 2 * r0:2 * (r0 + nr), :]
            lhs = _gated(u, tokens) if tokens else u
            m = _dot(lhs, bs[kk])
            if after is not None:
                after(i)
            return m

        m4 = prod(0, 3)
        m2 = prod(1, 1)
        hc[0, r0:r0 + nr, :] = _geglu(m2 + m4)
        m5 = prod(2, 4)
        m3 = prod(3, 2)
        hc[1, r0:r0 + nr, :] = _geglu(m3 + m5)
        m1 = prod(4, 0)
        ec[0, 2 * r0:2 * (r0 + nr), :] = (m4 - m5) + m1
        ec[1, 2 * r0:2 * (r0 + nr), :] = (m3 - m2) + m1

    init_state = {}

    def init_tile(t, tokens=None, lo=0, hi=D):
        if lo == 0:
            init_state['st'] = _Stats(4 if tokens is None else 1)
        st = init_state['st']
        for r in range(lo, hi, 16):
            x = qb[t, r:r + 16, :].astype(F32)
            x_s[t, r:r + 16, :] = x
            st.add(x[:8])
            st.add(x[8:])
            if tokens is not None and r % 32 == 16:
                e = st.s1[0] + st.s2[0]
                tokens.append(_token([e[:, j * BLK:(j + 1) * BLK] for j in range(TB)]))
        if hi < D:
            return None
        m, rs = st.finish()
        st0[t, 0:1, :] = m
        st0[t, 1:2, :] = rs
        return m, rs

    def tail(mid=None, after=None):
        def prod(i, kk, rhs):
            lhs = wdb[:DH, :FH] if kk == 2 else wdb[DH:, FH:] if kk == 3 else sd[kk]
            d = _dot(lhs, rhs.astype(BF16))
            if after is not None:
                after(i, d)
            return d

        m7 = _dot(sg[6], bs[6])
        h11 = _geglu(ec[0] + m7)
        m6 = _dot(sg[5], bs[5])
        h22 = _geglu(ec[1] + m6)
        if mid is not None:
            mid(m7, m6)
        h21, h12 = hc[0], hc[1]
        d2 = prod(0, 1, h11)
        d4 = prod(1, 3, h21 - h11)
        d6 = prod(2, 5, h11 + h12)
        d5 = prod(3, 4, h22)
        d1 = prod(4, 0, h11 + h22)
        d3 = prod(5, 2, h12 - h22)
        return d1, d2, d3, d4, d5, d6, lambda: prod(6, 6, h21 + h22)

    def residual(t, d):
        d1, d2, d3, d4, d5, d6, d7 = d
        d7 = d7()
        st = _Stats()
        for r in list(range(DH, D, 16)) + list(range(0, DH, 16)):
            if r < DH:
                q = slice(r, r + 16)
                f = jnp.concatenate([(d4[q] - d5[q]) + d1[q] + d7[q], d3[q] + d5[q]], axis=1)
            else:
                q = slice(r - DH, r - DH + 16)
                f = jnp.concatenate([d2[q] + d4[q], (d6[q] - d2[q]) + d1[q] + d3[q]], axis=1)
            xo = x_s[t, r:r + 16, :] + f
            ob[t, r:r + 16, :] = xo.astype(BF16)
            x_s[t, r:r + 16, :] = xo
            st.add(xo[:8])
            st.add(xo[8:])
        m, rs = st.finish()
        st0[t, 0:1, :] = m
        st0[t, 1:2, :] = rs

    def residual_last(d):
        t = NT - 1
        d1, d2, d3, d4, d5, d6, d7 = d
        ob[t, DH:, :] = (x_s[t, DH:, :] + jnp.concatenate(
            [d2 + d4, (d6 - d2) + d1 + d3], axis=1)).astype(BF16)
        ob[t, :DH, TH:] = (x_s[t, :DH, TH:] + (d3 + d5)).astype(BF16)
        e = x_s[t, :DH, :TH] + ((d4 - d5) + d1)
        d7 = d7()
        last_copy(0).start()
        last_copy(1).start()
        ob[t, :DH, :TH] = (e + d7).astype(BF16)
        last_copy(2).start()

    def prep_gate_up(c, tokens=None):
        combos = []
        for wbuf in (wgb, wub):
            blocks = []
            for half in range(2):
                t = wbuf[:, half * FH + c * BLK: half * FH + (c + 1) * BLK].astype(F32).T
                blocks.append(t[:, :KH])
                blocks.append(jnp.concatenate([t[:, KH:], jnp.zeros((BLK, 2 * KH - D), F32)],
                                              axis=1))
            combos.append(_a_combos(*blocks))
            if tokens is not None:
                e = combos[-1][0] + combos[-1][5]
                for r in range(0, BLK, 32):
                    tokens.append(_token([e[r + i:r + i + 8, j:j + BLK]
                                          for i in range(0, 32, 8) for j in range(0, KH, BLK)]))
        for kk in range(7):
            a = jnp.concatenate([combos[w][kk][16 * i:16 * i + 16]
                                 for i in range(BLK // 16) for w in range(2)], axis=0)
            sg[kk, 2 * c * BLK:2 * (c + 1) * BLK, :] = a.astype(BF16)

    def prep_down(lo, hi):
        tokens = []
        for r in range(lo, hi, 16):
            a11, a21 = (wdb[o + r:o + r + 16, :FH].astype(F32) for o in (0, DH))
            a12, a22 = (wdb[o + r:o + r + 16, FH:].astype(F32) for o in (0, DH))
            cs = _a_combos(a11, a12, a21, a22)
            for kk, a in enumerate(cs):
                if kk not in (2, 3):
                    sd[kk, r:r + 16, :] = a.astype(BF16)
            e = cs[0][:8] + cs[5][8:]
            tokens.append(_token([e[:, j * BLK:(j + 1) * BLK] for j in range(FH // BLK)]))
        return tokens

    parts = []
    for g in range(NC + 1):
        wait(c1_copies(g) if g < NC else [q_copy(0)])
        done, parts, tokens = parts, [], []
        if g > 0:
            for s in range(RC // 16):
                parts += conv_pairs((g - 1) * RC + s * 16, 0, tokens if g < NC else None)
        if g > 1:
            early, tokens = tokens[:N_EARLY], tokens[N_EARLY:]
            for n, z in enumerate(early):
                i = ((n // 2 + 1) * (RC // 16) // (N_EARLY // 2) - 1) * NH + (n % 2) * TB + TB - 1
                p = done[i]
                top = jnp.concatenate(
                    [p[:8, :BLK] + z.astype(jnp.int32).astype(F32), p[:8, BLK:]], axis=1)
                done[i] = jnp.concatenate([top, p[8:]], axis=0)
            conv_inv((g - 2) * RC, done, 0)
        if g < NC:
            conv_fwd(g * RC, RC, 0, conv_kv(g * RC, RC, 0), tokens)
    conv_inv((NC - 1) * RC, parts, 0)
    st = gate_layer(0, init_tile(0))
    wait(w_copies(0) + w_copies(1))
    ffn_operands(0, st)
    prep_gate_up(0)
    prep_gate_up(1)

    def prep_hook(chunks, wait_at):
        def before(i):
            tokens = []
            if i == wait_at:
                wait([c for g in chunks.values() for c in w_copies(g)])
            if i in chunks:
                prep_gate_up(chunks[i], tokens)
            return tokens
        return before

    def down_hook(i):
        tokens = []
        if i == 1:
            wait([wd_copy, q_copy(1)])
        if i > 0:
            tokens = prep_down((0, 48, 128, 176)[i - 1], (48, 128, 176, DH)[i - 1])
        if i in (2, 4):
            extra = []
            init_tile(1, extra, (i - 2) * DH // 2, i * DH // 2)
            tokens = [z for pair in zip(extra, tokens) for z in pair] + extra[len(tokens):]
        return tokens

    head(prep_hook({2: 2, 4: 3}, 2), None, 0, 2 * BLK)
    head(prep_hook({0: 4, 2: 5, 4: 6}, 0), None, 2 * BLK, 2 * BLK)
    head(down_hook, None, 4 * BLK, 3 * BLK)

    def tile_of(k):
        return 2 * (k // 4) + k % 2

    def step(k, with_conv):
        t_nxt = tile_of(k + 1)
        r0 = pl.multiple_of(k * R2_STRIDE, 16)
        box = {'d': []}

        def mid(m7, m6):
            st = (st0[t_nxt, 0:1, :], st0[t_nxt, 1:2, :])
            box['st'] = gate_layer(t_nxt, st, m7)
            if with_conv:
                box['kv'] = conv_kv(r0, R2, NH, m6)
            else:
                ffn_operands(t_nxt, box['st'], m6)

        def after_down(i, d):
            box['d'].append(d)
            if i == 2:
                ffn_operands(t_nxt, box['st'], jnp.concatenate(box['d'], axis=0))
                conv_fwd(r0, R2, NH, box['kv'])

        def before(i):
            tokens = []
            box['parts'] = []
            if i < len(PAIR_GROUPS):
                for s in range(PAIR_GROUPS[i]):
                    box['parts'] += conv_pairs(r0 + (sum(PAIR_GROUPS[:i]) + s) * 16, NH, tokens)
            else:
                init_tile(jnp.minimum(k + 2, NT - 1), tokens)
            return tokens

        def after(i):
            if box['parts']:
                conv_inv(r0 + sum(PAIR_GROUPS[:i]) * 16, box['parts'], NH)

        residual(tile_of(k), tail(mid, after_down if with_conv else None))
        if with_conv:
            head(before, after)
        else:
            head()

    def loop1(k, carry):
        for j in range(3):
            @pl.when(k == j)
            def _():
                wait(c2_copies(j))
        step(k, True)
        return carry

    def loop2(k, carry):
        step(k, False)
        for kk, t in ((3, 1), (6, 2)):
            @pl.when(k == kk)
            def _():
                o_copy(t).start()
        return carry

    lax.fori_loop(0, 3, loop1, 0)
    o_copy(0).start()
    lax.fori_loop(3, 7, loop2, 0)
    residual_last(tail())
    wait([o_copy(t) for t in range(NT - 1)] + [last_copy(n) for n in range(3)])


@jax.jit
def pallas_interleave_layers__ssm_conv_h3__geglu_ffn__prompt_kernel(A_q, A_k, A_v, A_shift_k, A_ssm_k, A_ssm_D, B_x, B_w_gate, B_w_up, B_w_down):
    ft, gi = _dft_consts()
    anyspec = pl.BlockSpec(memory_space=pl.ANY)
    vm = pltpu.VMEM
    out_t = pl.pallas_call(
        _kernel,
        in_specs=[anyspec] * 11,
        out_specs=anyspec,
        out_shape=jax.ShapeDtypeStruct((D, S), BF16),
        scratch_shapes=[
            vm((NT, D, TM), BF16), vm((D, S), BF16), vm((D, S), BF16), vm((D, S), BF16),
            vm((4, D), BF16), vm((D,), BF16),
            vm((D, F), BF16), vm((D, F), BF16), vm((D, F), BF16),
            vm((BLK, 2 * BLK), BF16), vm((2 * BLK, BLK), BF16),
            vm((7, F, KH), BF16), vm((7, DH, FH), BF16),
            vm((5, D, BLK), F32),
            vm((3, NB, D, BLK), F32), vm((3, NB, D, BLK), F32), vm((D, 2 * BLK), F32),
            vm((NT, D, TM), F32), vm((NT, D, TM), F32), vm((NT, 8, TM), F32),
            vm((7, KH, TH), BF16), vm((2, F, TH), F32), vm((2, FH, TH), F32),
            vm((NT, D, TM), BF16),
            pltpu.SemaphoreType.DMA((NUM_SEMS,)), pltpu.SemaphoreType.REGULAR,
        ],
        compiler_params=pltpu.CompilerParams(vmem_limit_bytes=110 * 1024 * 1024),
    )(A_q[0].T, A_k[0].T, A_v[0].T, A_shift_k.T, A_ssm_k, A_ssm_D,
      B_w_gate, B_w_up, B_w_down.T, ft, gi)
    return out_t.T[None]
```

```python
import numpy as np
import jax
import jax.numpy as jnp
from jax import lax
import jax.experimental.pallas as pl
import jax.experimental.pallas.tpu as pltpu

S, D, F = 2048, 448, 1792
BLK = 128
NB = S // BLK
NH = NB // 2
SH = S // 2
TM = 512
TB = TM // BLK
TH = TM // 2
NT = S // TM
FH = F // 2
DH = D // 2
KH = 256
NC = 7
RC = D // NC
R2 = 160
R2_STRIDE = 144
C2_ROWS = ((0, 160), (160, 144), (304, 144))
PAIR_GROUPS = (3, 2, 3, 2)
PAIR_SKIPS = (128, 128, 128, 128, 0)
N_EARLY = 8
SEM_C2 = NC
SEM_W01, SEM_W23, SEM_W46, SEM_Q0, SEM_WD, SEM_SMALL, SEM_OUT = (NC + 3 + i for i in range(7))
NUM_SEMS = NC + 10
EPS = 1e-5
HUGE = 3.0e38
F32 = jnp.float32
BF16 = jnp.bfloat16
U32 = jnp.uint32
XN_SCALE = float(np.sqrt(0.5))
GELU_C0 = float(np.sqrt(2.0 / np.pi)) / XN_SCALE
GELU_C1 = float(np.sqrt(2.0 / np.pi)) * 0.044715 / XN_SCALE ** 3


def _dft_consts():
    n = np.arange(BLK)[:, None]
    m = np.arange(BLK)[None, :]
    ang = np.pi * (((4 * m + 1) * n) % 512) / 256.0
    ft = np.concatenate([np.cos(ang), -np.sin(ang)], axis=1)
    gi = ft.T / BLK
    return jnp.asarray(ft, BF16), jnp.asarray(gi, BF16)


class _Stats:
    def __init__(self, ways=1):
        self.c = None
        self.n = 0
        self.s1 = [None] * ways
        self.s2 = [None] * ways

    def add(self, x):
        if self.c is None:
            self.c = x[0:1, :]
        xs = x - self.c
        w = self.n % len(self.s1)
        self.n += 1
        self.s1[w] = xs if self.s1[w] is None else self.s1[w] + xs
        self.s2[w] = xs * xs if self.s2[w] is None else self.s2[w] + xs * xs

    def finish(self):
        def tree(v):
            while len(v) > 1:
                v = [v[i] + v[i + 1] for i in range(0, len(v), 2)]
            return v[0]
        m = jnp.sum(tree(self.s1), axis=0, keepdims=True) * (1.0 / D)
        v = jnp.sum(tree(self.s2), axis=0, keepdims=True) * (1.0 / D) - m * m
        return self.c + m, lax.rsqrt(jnp.maximum(v, 0.0) + EPS)


def _a_combos(a11, a12, a21, a22):
    return [a11 + a22, a21 + a22, a11, a22, a11 + a12, a21 - a11, a12 - a22]


def _b_combos(b11, b12, b21, b22):
    return [b11 + b22, b11, b12 - b22, b21 - b11, b22, b11 + b12, b21 + b22]


def _geglu(c):
    n = c.shape[0] // 32
    g = jnp.concatenate([c[32 * i:32 * i + 16] for i in range(n)], axis=0)
    u = jnp.concatenate([c[32 * i + 16:32 * i + 32] for i in range(n)], axis=0)
    t = jnp.tanh(g * (GELU_C0 + GELU_C1 * (g * g)))
    gu = g * u
    return gu + gu * t


def _dot(a, b):
    return jnp.dot(a, b, preferred_element_type=F32)


def _tick(pace, i, n):
    if pace is None:
        return None
    r = (i * pace.shape[0] // n) // 8 * 8
    return jnp.where(pace[r:r + 8, :BLK] > HUGE, 1.0, 0.0)


def _after(x, z):
    if z is None:
        return x
    return x + jnp.tile(z, (x.shape[0] // 8, x.shape[1] // BLK))


def _token(vals):
    acc = vals[0]
    for v in vals[1:]:
        acc = acc + v
    return jnp.where(acc > HUGE, jnp.uint32(1), jnp.uint32(0))


def _gated(u, tokens, skip=0):
    n = len(tokens)
    pieces, prev = [], 0
    for i, z in enumerate(tokens):
        p = (skip + (i + 1) * (u.shape[0] - skip) // n) // 16 * 16 - 16
        seg = u[p:p + 16]
        pieces += [u[prev:p]] if p > prev else []
        first = pltpu.bitcast(pltpu.bitcast(seg[:, :BLK], U32) | z, BF16)
        pieces.append(jnp.concatenate([first, seg[:, BLK:]], axis=1) if u.shape[1] > BLK else first)
        prev = p + 16
    if prev < u.shape[0]:
        pieces.append(u[prev:])
    return jnp.concatenate(pieces, axis=0)


def _kernel(q_hbm, k_hbm, v_hbm, sk_hbm, h_hbm, d_hbm, wg_hbm, wu_hbm, wd_hbm, ft_hbm, gi_hbm,
            o_hbm,
            qb, kb, vb, hb, skb, db, wgb, wub, wdb, ftb, gib,
            sg, sd, par, up, hp, hraw, y_s, x_s, st0, bs, ec, hc, ob,
            sems, sem_f):
    kvh = ((k_hbm, kb), (v_hbm, vb), (h_hbm, hb))

    def fence():
        pl.semaphore_signal(sem_f, 1)
        pl.semaphore_wait(sem_f, 1)

    def c1_copies(g):
        rows, cols = pl.ds(g * RC, RC), pl.ds(0, SH)
        return [pltpu.make_async_copy(src.at[rows, cols], dst.at[rows, cols], sems.at[g])
                for src, dst in kvh]

    def c2_copies(j):
        rows, cols = pl.ds(*C2_ROWS[j]), pl.ds(SH, SH)
        cs = [pltpu.make_async_copy(src.at[rows, cols], dst.at[rows, cols], sems.at[SEM_C2 + j])
              for src, dst in kvh]
        return cs + ([q_copy(2 + j)] if j < 2 else [])

    def w_copies(g):
        sem = sems.at[(SEM_W01, SEM_W01, SEM_W23, SEM_W23, SEM_W46, SEM_W46, SEM_W46)[g]]
        cs = []
        for src, dst in ((wg_hbm, wgb), (wu_hbm, wub)):
            for half in range(2):
                cols = pl.ds(half * FH + g * BLK, BLK)
                cs.append(pltpu.make_async_copy(src.at[:, cols], dst.at[:, cols], sem))
        return cs

    def q_copy(t):
        sem = sems.at[(SEM_Q0, SEM_WD, SEM_C2, SEM_C2 + 1)[t]]
        return pltpu.make_async_copy(q_hbm.at[:, pl.ds(t * TM, TM)], qb.at[t], sem)

    wd_copy = pltpu.make_async_copy(wd_hbm, wdb, sems.at[SEM_WD])

    def o_copy(t):
        return pltpu.make_async_copy(ob.at[t], o_hbm.at[:, pl.ds(t * TM, TM)], sems.at[SEM_OUT])

    def last_copy(n):
        rows, cols = ((pl.ds(DH, DH), pl.ds(0, TM)), (pl.ds(0, DH), pl.ds(TH, TH)),
                      (pl.ds(0, DH), pl.ds(0, TH)))[n]
        dst = pl.ds((NT - 1) * TM + cols.start, cols.size)
        return pltpu.make_async_copy(ob.at[NT - 1, rows, cols], o_hbm.at[rows, dst],
                                     sems.at[SEM_OUT])

    small = [pltpu.make_async_copy(s, d, sems.at[SEM_SMALL]) for s, d in
             ((sk_hbm, skb), (d_hbm, db), (ft_hbm, ftb), (gi_hbm, gib))]

    def wait(copies):
        for c in copies:
            c.wait()

    for group in ([small] + [c1_copies(g) for g in range(NC)] + [[q_copy(0)]]
                  + [w_copies(g) for g in range(NC)] + [[wd_copy], [q_copy(1)]]
                  + [c2_copies(j) for j in range(3)]):
        for c in group:
            c.start()
        fence()

    wait(small)
    sk = skb[...].astype(F32)
    for t in range(4):
        par[t] = jnp.broadcast_to(sk[t:t + 1, :], (BLK, D)).T
    par[4] = jnp.broadcast_to(db[...].astype(F32).reshape(1, D), (BLK, D)).T

    def conv_kv(r0, nrows, b0, pace=None):
        first = b0 == 0
        off = 0 if first else BLK
        parts = []
        for s in range(nrows // 16):
            rows = pl.ds(r0 + s * 16, 16)
            kf = _after(kb[rows, b0 * BLK - off:(b0 + NH) * BLK].astype(F32),
                        _tick(pace, s, nrows // 16))
            nw = NH + off // BLK
            acc = kf[:, off:] * jnp.tile(par[0, rows, :], (1, NH))
            for t in range(1, 4):
                sh = pltpu.roll(kf * jnp.tile(par[t, rows, :], (1, nw)), t, 1)[:, off:]
                if first:
                    lane = lax.broadcasted_iota(jnp.int32, (16, BLK), 1)
                    sh = jnp.concatenate([jnp.where(lane >= t, sh[:, :BLK], 0.0), sh[:, BLK:]],
                                         axis=1)
                acc = acc + sh
            kv = acc * vb[rows, b0 * BLK:(b0 + NH) * BLK].astype(F32)
            parts += [kv[:, a * BLK:(a + 1) * BLK] for a in range(NH)]
        return jnp.concatenate(parts, axis=0).astype(BF16)

    def conv_fwd(r0, nrows, b0, kv, tokens=None):
        first = b0 == 0
        hs = hb[pl.ds(r0, nrows), b0 * BLK:(b0 + NH) * BLK]
        hst = jnp.concatenate([hs[s:s + 16, a * BLK:(a + 1) * BLK]
                               for s in range(0, nrows, 16) for a in range(NH)], axis=0)
        if tokens:
            hst = _gated(hst, tokens)
        hf = _dot(hst, ftb[...])
        uf = _dot(kv, ftb[...])
        for gg in range(nrows // 8):
            r8 = pl.ds(r0 + gg * 8, 8)
            zp = None if first else hraw[r8, :]
            us, hs = [], []
            for a in range(NH):
                base = (gg // 2) * 16 * NH + a * 16 + (gg % 2) * 8
                z = uf[base:base + 8, :]
                ur, ui = z[:, :BLK], z[:, BLK:]
                us.append((ur + ui, ur, ui))
                z = hf[base:base + 8, :]
                if zp is None:
                    c = z[:, :BLK] + par[4, r8, :]
                    d = z[:, BLK:]
                else:
                    c = z[:, :BLK] - zp[:, BLK:]
                    d = z[:, BLK:] + zp[:, :BLK]
                hs.append((c, d - c, c + d))
                zp = z
            for p in range(3):
                up[p, b0:b0 + NH, r8, :] = jnp.stack([t[p] for t in us])
                hp[p, b0:b0 + NH, r8, :] = jnp.stack([t[p] for t in hs])
            if first:
                hraw[r8, :] = zp

    def conv_pairs(r0, b0, tokens=None):
        b1 = b0 + NH
        ks = []
        for p in range(3):
            kp = []
            for gg in range(2):
                r8 = pl.ds(r0 + gg * 8, 8)
                uu = up[p, :b1, r8, :]
                hh = hp[p, :b1, r8, :]
                ka = []
                for a in range(b0, b1):
                    acc = hh[0] * uu[a]
                    for j in range(1, a + 1):
                        acc = acc + hh[j] * uu[a - j]
                    ka.append(acc)
                kp.append(ka)
                if tokens is not None:
                    tokens.append(_token(ka))
            ks.append([jnp.concatenate([kp[0][a], kp[1][a]], axis=0) for a in range(NH)])
        return [jnp.concatenate([ks[0][a] - ks[2][a], ks[0][a] + ks[1][a]], axis=1)
                for a in range(NH)]

    def conv_inv(r0, parts, b0):
        ns = len(parts) // NH
        for tt in range(NH // TB):
            lhs = jnp.concatenate(
                [parts[s * NH + tt * TB + a] for s in range(ns) for a in range(TB)], axis=0)
            yt = _dot(lhs.astype(BF16), gib[...])
            cols = [jnp.concatenate(
                [yt[(s * TB + a) * 16:(s * TB + a + 1) * 16, :] for s in range(ns)], axis=0)
                for a in range(TB)]
            y_s[b0 // TB + tt, pl.ds(r0, ns * 16), :] = jnp.concatenate(cols, axis=1)

    def gate_layer(t, stats, pace=None):
        m, rs = stats
        st = _Stats(4)
        for r in range(0, D, 8):
            if r % 16 == 0:
                mb = _after(jnp.broadcast_to(m, (8, TM)), _tick(pace, r // 16, D // 16))
            x = x_s[t, r:r + 8, :]
            x1 = x + (x - mb) * rs * y_s[t, r:r + 8, :]
            x_s[t, r:r + 8, :] = x1
            st.add(x1)
        return st.finish()

    def ffn_operands(t, stats, pace=None):
        m, rs = stats
        rs = rs * XN_SCALE
        for r in range(0, KH, 16):
            mb = _after(jnp.broadcast_to(m, (8, TM)), _tick(pace, r // 16, KH // 16))
            mb = jnp.concatenate([mb, mb], axis=0)
            hi = (x_s[t, r:r + 16, :] - mb) * rs
            if KH + r < D:
                lo = (x_s[t, KH + r:KH + r + 16, :] - mb) * rs
            else:
                lo = jnp.zeros((16, TM), F32)
            for kk, b in enumerate(_b_combos(hi[:, :TH], hi[:, TH:], lo[:, :TH], lo[:, TH:])):
                bs[kk, r:r + 16, :] = b.astype(BF16)

    def head(before=None, after=None, r0=0, nr=FH):
        def prod(i, kk):
            tokens = before(i) if before is not None else None
            u = sg[kk, 2 * r0:2 * (r0 + nr), :]
            lhs = _gated(u, tokens, PAIR_SKIPS[i] if nr == FH else 0) if tokens else u
            m = _dot(lhs, bs[kk])
            if after is not None:
                after(i)
            return m

        m4 = prod(0, 3)
        m2 = prod(1, 1)
        hc[0, r0:r0 + nr, :] = _geglu(m2 + m4)
        m5 = prod(2, 4)
        m3 = prod(3, 2)
        hc[1, r0:r0 + nr, :] = _geglu(m3 + m5)
        m1 = prod(4, 0)
        ec[0, 2 * r0:2 * (r0 + nr), :] = (m4 - m5) + m1
        ec[1, 2 * r0:2 * (r0 + nr), :] = (m3 - m2) + m1

    init_state = {}

    def init_tile(t, tokens=None, lo=0, hi=D):
        if lo == 0:
            init_state['st'] = _Stats(4 if tokens is None else 1)
        st = init_state['st']
        for r in range(lo, hi, 16):
            x = qb[t, r:r + 16, :].astype(F32)
            x_s[t, r:r + 16, :] = x
            st.add(x[:8])
            st.add(x[8:])
            if tokens is not None and r % 32 == 16:
                e = st.s1[0] + st.s2[0]
                tokens.append(_token([e[:, j * BLK:(j + 1) * BLK] for j in range(TB)]))
        if hi < D:
            return None
        m, rs = st.finish()
        st0[t, 0:1, :] = m
        st0[t, 1:2, :] = rs
        return m, rs

    def tail(mid=None, after=None):
        def prod(i, kk, rhs):
            lhs = wdb[:DH, :FH] if kk == 2 else wdb[DH:, FH:] if kk == 3 else sd[kk]
            d = _dot(lhs, rhs.astype(BF16))
            if after is not None:
                after(i, d)
            return d

        m7 = _dot(sg[6], bs[6])
        h11 = _geglu(ec[0] + m7)
        m6 = _dot(sg[5], bs[5])
        h22 = _geglu(ec[1] + m6)
        if mid is not None:
            mid(m7, m6)
        h21, h12 = hc[0], hc[1]
        d2 = prod(0, 1, h11)
        d4 = prod(1, 3, h21 - h11)
        d6 = prod(2, 5, h11 + h12)
        d5 = prod(3, 4, h22)
        d1 = prod(4, 0, h11 + h22)
        d3 = prod(5, 2, h12 - h22)
        return d1, d2, d3, d4, d5, d6, lambda: prod(6, 6, h21 + h22)

    def residual(t, d):
        d1, d2, d3, d4, d5, d6, d7 = d
        d7 = d7()
        st = _Stats()
        for r in list(range(DH, D, 16)) + list(range(0, DH, 16)):
            if r < DH:
                q = slice(r, r + 16)
                f = jnp.concatenate([(d4[q] - d5[q]) + d1[q] + d7[q], d3[q] + d5[q]], axis=1)
            else:
                q = slice(r - DH, r - DH + 16)
                f = jnp.concatenate([d2[q] + d4[q], (d6[q] - d2[q]) + d1[q] + d3[q]], axis=1)
            xo = x_s[t, r:r + 16, :] + f
            ob[t, r:r + 16, :] = xo.astype(BF16)
            x_s[t, r:r + 16, :] = xo
            st.add(xo[:8])
            st.add(xo[8:])
        m, rs = st.finish()
        st0[t, 0:1, :] = m
        st0[t, 1:2, :] = rs

    def residual_last(d):
        t = NT - 1
        d1, d2, d3, d4, d5, d6, d7 = d
        ob[t, DH:, :] = (x_s[t, DH:, :] + jnp.concatenate(
            [d2 + d4, (d6 - d2) + d1 + d3], axis=1)).astype(BF16)
        ob[t, :DH, TH:] = (x_s[t, :DH, TH:] + (d3 + d5)).astype(BF16)
        e = x_s[t, :DH, :TH] + ((d4 - d5) + d1)
        d7 = d7()
        last_copy(0).start()
        last_copy(1).start()
        ob[t, :DH, :TH] = (e + d7).astype(BF16)
        last_copy(2).start()

    def prep_gate_up(c, tokens=None):
        combos = []
        for wbuf in (wgb, wub):
            blocks = []
            for half in range(2):
                t = wbuf[:, half * FH + c * BLK: half * FH + (c + 1) * BLK].astype(F32).T
                blocks.append(t[:, :KH])
                blocks.append(jnp.concatenate([t[:, KH:], jnp.zeros((BLK, 2 * KH - D), F32)],
                                              axis=1))
            combos.append(_a_combos(*blocks))
            if tokens is not None:
                e = combos[-1][0] + combos[-1][5]
                for r in range(0, BLK, 32):
                    tokens.append(_token([e[r + i:r + i + 8, j:j + BLK]
                                          for i in range(0, 32, 8) for j in range(0, KH, BLK)]))
        for kk in range(7):
            a = jnp.concatenate([combos[w][kk][16 * i:16 * i + 16]
                                 for i in range(BLK // 16) for w in range(2)], axis=0)
            sg[kk, 2 * c * BLK:2 * (c + 1) * BLK, :] = a.astype(BF16)

    def prep_down(lo, hi):
        tokens = []
        for r in range(lo, hi, 16):
            a11, a21 = (wdb[o + r:o + r + 16, :FH].astype(F32) for o in (0, DH))
            a12, a22 = (wdb[o + r:o + r + 16, FH:].astype(F32) for o in (0, DH))
            cs = _a_combos(a11, a12, a21, a22)
            for kk, a in enumerate(cs):
                if kk not in (2, 3):
                    sd[kk, r:r + 16, :] = a.astype(BF16)
            e = cs[0][:8] + cs[5][8:]
            tokens.append(_token([e[:, j * BLK:(j + 1) * BLK] for j in range(FH // BLK)]))
        return tokens

    parts = []
    for g in range(NC + 1):
        wait(c1_copies(g) if g < NC else [q_copy(0)])
        done, parts, tokens = parts, [], []
        if g > 0:
            for s in range(RC // 16):
                parts += conv_pairs((g - 1) * RC + s * 16, 0, tokens if g < NC else None)
        if g > 1:
            early, tokens = tokens[:N_EARLY], tokens[N_EARLY:]
            for n, z in enumerate(early):
                i = ((n // 2 + 1) * (RC // 16) // (N_EARLY // 2) - 1) * NH + (n % 2) * TB + TB - 1
                p = done[i]
                top = jnp.concatenate(
                    [p[:8, :BLK] + z.astype(jnp.int32).astype(F32), p[:8, BLK:]], axis=1)
                done[i] = jnp.concatenate([top, p[8:]], axis=0)
            conv_inv((g - 2) * RC, done, 0)
        if g < NC:
            conv_fwd(g * RC, RC, 0, conv_kv(g * RC, RC, 0), tokens)
    conv_inv((NC - 1) * RC, parts, 0)
    st = gate_layer(0, init_tile(0))
    wait(w_copies(0) + w_copies(1))
    ffn_operands(0, st)
    prep_gate_up(0)
    prep_gate_up(1)

    def prep_hook(chunks, wait_at):
        def before(i):
            tokens = []
            if i == wait_at:
                wait([c for g in chunks.values() for c in w_copies(g)])
            if i in chunks:
                prep_gate_up(chunks[i], tokens)
            return tokens
        return before

    def down_hook(i):
        tokens = []
        if i == 1:
            wait([wd_copy, q_copy(1)])
        if i > 0:
            tokens = prep_down((0, 48, 128, 176)[i - 1], (48, 128, 176, DH)[i - 1])
        if i in (2, 4):
            extra = []
            init_tile(1, extra, (i - 2) * DH // 2, i * DH // 2)
            tokens = [z for pair in zip(extra, tokens) for z in pair] + extra[len(tokens):]
        return tokens

    head(prep_hook({2: 2, 4: 3}, 2), None, 0, 2 * BLK)
    head(prep_hook({0: 4, 2: 5, 4: 6}, 0), None, 2 * BLK, 2 * BLK)
    head(down_hook, None, 4 * BLK, 3 * BLK)

    def tile_of(k):
        return 2 * (k // 4) + k % 2

    def step(k, with_conv):
        t_nxt = tile_of(k + 1)
        r0 = pl.multiple_of(k * R2_STRIDE, 16)
        box = {'d': []}

        def mid(m7, m6):
            st = (st0[t_nxt, 0:1, :], st0[t_nxt, 1:2, :])
            box['st'] = gate_layer(t_nxt, st, m7)
            if with_conv:
                box['kv'] = conv_kv(r0, R2, NH, m6)
            else:
                ffn_operands(t_nxt, box['st'], m6)

        def after_down(i, d):
            box['d'].append(d)
            if i == 2:
                ffn_operands(t_nxt, box['st'], jnp.concatenate(box['d'], axis=0))
                conv_fwd(r0, R2, NH, box['kv'])

        def before(i):
            tokens = []
            box['parts'] = []
            if i < len(PAIR_GROUPS):
                for s in range(PAIR_GROUPS[i]):
                    box['parts'] += conv_pairs(r0 + (sum(PAIR_GROUPS[:i]) + s) * 16, NH, tokens)
            else:
                init_tile(jnp.minimum(k + 2, NT - 1), tokens)
            return tokens

        def after(i):
            if box['parts']:
                conv_inv(r0 + sum(PAIR_GROUPS[:i]) * 16, box['parts'], NH)

        residual(tile_of(k), tail(mid, after_down if with_conv else None))
        if with_conv:
            head(before, after)
        else:
            head()

    def loop1(k, carry):
        for j in range(3):
            @pl.when(k == j)
            def _():
                wait(c2_copies(j))
        step(k, True)
        return carry

    def loop2(k, carry):
        step(k, False)
        for kk, t in ((3, 1), (6, 2)):
            @pl.when(k == kk)
            def _():
                o_copy(t).start()
        return carry

    lax.fori_loop(0, 3, loop1, 0)
    o_copy(0).start()
    lax.fori_loop(3, 7, loop2, 0)
    residual_last(tail())
    wait([o_copy(t) for t in range(NT - 1)] + [last_copy(n) for n in range(3)])


@jax.jit
def pallas_interleave_layers__ssm_conv_h3__geglu_ffn__prompt_kernel(A_q, A_k, A_v, A_shift_k, A_ssm_k, A_ssm_D, B_x, B_w_gate, B_w_up, B_w_down):
    ft, gi = _dft_consts()
    anyspec = pl.BlockSpec(memory_space=pl.ANY)
    vm = pltpu.VMEM
    out_t = pl.pallas_call(
        _kernel,
        in_specs=[anyspec] * 11,
        out_specs=anyspec,
        out_shape=jax.ShapeDtypeStruct((D, S), BF16),
        scratch_shapes=[
            vm((NT, D, TM), BF16), vm((D, S), BF16), vm((D, S), BF16), vm((D, S), BF16),
            vm((4, D), BF16), vm((D,), BF16),
            vm((D, F), BF16), vm((D, F), BF16), vm((D, F), BF16),
            vm((BLK, 2 * BLK), BF16), vm((2 * BLK, BLK), BF16),
            vm((7, F, KH), BF16), vm((7, DH, FH), BF16),
            vm((5, D, BLK), F32),
            vm((3, NB, D, BLK), F32), vm((3, NB, D, BLK), F32), vm((D, 2 * BLK), F32),
            vm((NT, D, TM), F32), vm((NT, D, TM), F32), vm((NT, 8, TM), F32),
            vm((7, KH, TH), BF16), vm((2, F, TH), F32), vm((2, FH, TH), F32),
            vm((NT, D, TM), BF16),
            pltpu.SemaphoreType.DMA((NUM_SEMS,)), pltpu.SemaphoreType.REGULAR,
        ],
        compiler_params=pltpu.CompilerParams(vmem_limit_bytes=110 * 1024 * 1024),
    )(A_q[0].T, A_k[0].T, A_v[0].T, A_shift_k.T, A_ssm_k, A_ssm_D,
      B_w_gate, B_w_up, B_w_down.T, ft, gi)
    return out_t.T[None]
```

```python
import numpy as np
import jax
import jax.numpy as jnp
from jax import lax
import jax.experimental.pallas as pl
import jax.experimental.pallas.tpu as pltpu

S, D, F = 2048, 448, 1792
BLK = 128
NB = S // BLK
NH = NB // 2
SH = S // 2
TM = 512
TB = TM // BLK
TH = TM // 2
NT = S // TM
FH = F // 2
DH = D // 2
KH = 256
NC = 7
RC = D // NC
R2 = 160
R2_STRIDE = 144
C2_ROWS = ((0, 160), (160, 144), (304, 144))
PAIR_GROUPS = (3, 2, 3, 2)
PAIR_SKIPS = (384, 192, 192, 192, 0)
N_EARLY = 8
SEM_C2 = NC
SEM_W01, SEM_W23, SEM_W46, SEM_Q0, SEM_WD, SEM_SMALL, SEM_OUT = (NC + 3 + i for i in range(7))
NUM_SEMS = NC + 10
EPS = 1e-5
HUGE = 3.0e38
F32 = jnp.float32
BF16 = jnp.bfloat16
U32 = jnp.uint32
XN_SCALE = float(np.sqrt(0.5))
GELU_C0 = float(np.sqrt(2.0 / np.pi)) / XN_SCALE
GELU_C1 = float(np.sqrt(2.0 / np.pi)) * 0.044715 / XN_SCALE ** 3


def _dft_consts():
    n = np.arange(BLK)[:, None]
    m = np.arange(BLK)[None, :]
    ang = np.pi * (((4 * m + 1) * n) % 512) / 256.0
    ft = np.concatenate([np.cos(ang), -np.sin(ang)], axis=1)
    gi = ft.T / BLK
    return jnp.asarray(ft, BF16), jnp.asarray(gi, BF16)


class _Stats:
    def __init__(self, ways=1):
        self.c = None
        self.n = 0
        self.s1 = [None] * ways
        self.s2 = [None] * ways

    def add(self, x):
        if self.c is None:
            self.c = x[0:1, :]
        xs = x - self.c
        w = self.n % len(self.s1)
        self.n += 1
        self.s1[w] = xs if self.s1[w] is None else self.s1[w] + xs
        self.s2[w] = xs * xs if self.s2[w] is None else self.s2[w] + xs * xs

    def finish(self):
        def tree(v):
            while len(v) > 1:
                v = [v[i] + v[i + 1] for i in range(0, len(v), 2)]
            return v[0]
        m = jnp.sum(tree(self.s1), axis=0, keepdims=True) * (1.0 / D)
        v = jnp.sum(tree(self.s2), axis=0, keepdims=True) * (1.0 / D) - m * m
        return self.c + m, lax.rsqrt(jnp.maximum(v, 0.0) + EPS)


def _a_combos(a11, a12, a21, a22):
    return [a11 + a22, a21 + a22, a11, a22, a11 + a12, a21 - a11, a12 - a22]


def _b_combos(b11, b12, b21, b22):
    return [b11 + b22, b11, b12 - b22, b21 - b11, b22, b11 + b12, b21 + b22]


def _geglu(c):
    n = c.shape[0] // 32
    g = jnp.concatenate([c[32 * i:32 * i + 16] for i in range(n)], axis=0)
    u = jnp.concatenate([c[32 * i + 16:32 * i + 32] for i in range(n)], axis=0)
    t = jnp.tanh(g * (GELU_C0 + GELU_C1 * (g * g)))
    gu = g * u
    return gu + gu * t


def _dot(a, b):
    return jnp.dot(a, b, preferred_element_type=F32)


def _tick(pace, i, n):
    if pace is None:
        return None
    r = (i * pace.shape[0] // n) // 8 * 8
    return jnp.where(pace[r:r + 8, :BLK] > HUGE, 1.0, 0.0)


def _after(x, z):
    if z is None:
        return x
    return x + jnp.tile(z, (x.shape[0] // 8, x.shape[1] // BLK))


def _token(vals):
    acc = vals[0]
    for v in vals[1:]:
        acc = acc + v
    return jnp.where(acc > HUGE, jnp.uint32(1), jnp.uint32(0))


def _gated(u, tokens, skip=0):
    n = len(tokens)
    pieces, prev = [], 0
    for i, z in enumerate(tokens):
        p = (skip + (i + 1) * (u.shape[0] - skip) // n) // 16 * 16 - 16
        seg = u[p:p + 16]
        pieces += [u[prev:p]] if p > prev else []
        first = pltpu.bitcast(pltpu.bitcast(seg[:, :BLK], U32) | z, BF16)
        pieces.append(jnp.concatenate([first, seg[:, BLK:]], axis=1) if u.shape[1] > BLK else first)
        prev = p + 16
    if prev < u.shape[0]:
        pieces.append(u[prev:])
    return jnp.concatenate(pieces, axis=0)


def _kernel(q_hbm, k_hbm, v_hbm, sk_hbm, h_hbm, d_hbm, wg_hbm, wu_hbm, wd_hbm, ft_hbm, gi_hbm,
            o_hbm,
            qb, kb, vb, hb, skb, db, wgb, wub, wdb, ftb, gib,
            sg, sd, par, up, hp, hraw, y_s, x_s, st0, bs, ec, hc, ob,
            sems, sem_f):
    kvh = ((k_hbm, kb), (v_hbm, vb), (h_hbm, hb))

    def fence():
        pl.semaphore_signal(sem_f, 1)
        pl.semaphore_wait(sem_f, 1)

    def c1_copies(g):
        rows, cols = pl.ds(g * RC, RC), pl.ds(0, SH)
        return [pltpu.make_async_copy(src.at[rows, cols], dst.at[rows, cols], sems.at[g])
                for src, dst in kvh]

    def c2_copies(j):
        rows, cols = pl.ds(*C2_ROWS[j]), pl.ds(SH, SH)
        cs = [pltpu.make_async_copy(src.at[rows, cols], dst.at[rows, cols], sems.at[SEM_C2 + j])
              for src, dst in kvh]
        return cs + ([q_copy(2 + j)] if j < 2 else [])

    def w_copies(g):
        sem = sems.at[(SEM_W01, SEM_W01, SEM_W23, SEM_W23, SEM_W46, SEM_W46, SEM_W46)[g]]
        cs = []
        for src, dst in ((wg_hbm, wgb), (wu_hbm, wub)):
            for half in range(2):
                cols = pl.ds(half * FH + g * BLK, BLK)
                cs.append(pltpu.make_async_copy(src.at[:, cols], dst.at[:, cols], sem))
        return cs

    def q_copy(t):
        sem = sems.at[(SEM_Q0, SEM_WD, SEM_C2, SEM_C2 + 1)[t]]
        return pltpu.make_async_copy(q_hbm.at[:, pl.ds(t * TM, TM)], qb.at[t], sem)

    wd_copy = pltpu.make_async_copy(wd_hbm, wdb, sems.at[SEM_WD])

    def o_copy(t):
        return pltpu.make_async_copy(ob.at[t], o_hbm.at[:, pl.ds(t * TM, TM)], sems.at[SEM_OUT])

    def last_copy(n):
        rows, cols = ((pl.ds(DH, DH), pl.ds(0, TM)), (pl.ds(0, DH), pl.ds(TH, TH)),
                      (pl.ds(0, DH), pl.ds(0, TH)))[n]
        dst = pl.ds((NT - 1) * TM + cols.start, cols.size)
        return pltpu.make_async_copy(ob.at[NT - 1, rows, cols], o_hbm.at[rows, dst],
                                     sems.at[SEM_OUT])

    small = [pltpu.make_async_copy(s, d, sems.at[SEM_SMALL]) for s, d in
             ((sk_hbm, skb), (d_hbm, db), (ft_hbm, ftb), (gi_hbm, gib))]

    def wait(copies):
        for c in copies:
            c.wait()

    for group in ([small] + [c1_copies(g) for g in range(NC)] + [[q_copy(0)]]
                  + [w_copies(g) for g in range(NC)] + [[wd_copy], [q_copy(1)]]
                  + [c2_copies(j) for j in range(3)]):
        for c in group:
            c.start()
        fence()

    wait(small)
    sk = skb[...].astype(F32)
    for t in range(4):
        par[t] = jnp.broadcast_to(sk[t:t + 1, :], (BLK, D)).T
    par[4] = jnp.broadcast_to(db[...].astype(F32).reshape(1, D), (BLK, D)).T

    def conv_kv(r0, nrows, b0, pace=None):
        first = b0 == 0
        off = 0 if first else BLK
        parts = []
        for s in range(nrows // 16):
            rows = pl.ds(r0 + s * 16, 16)
            kf = _after(kb[rows, b0 * BLK - off:(b0 + NH) * BLK].astype(F32),
                        _tick(pace, s, nrows // 16))
            nw = NH + off // BLK
            acc = kf[:, off:] * jnp.tile(par[0, rows, :], (1, NH))
            for t in range(1, 4):
                sh = pltpu.roll(kf * jnp.tile(par[t, rows, :], (1, nw)), t, 1)[:, off:]
                if first:
                    lane = lax.broadcasted_iota(jnp.int32, (16, BLK), 1)
                    sh = jnp.concatenate([jnp.where(lane >= t, sh[:, :BLK], 0.0), sh[:, BLK:]],
                                         axis=1)
                acc = acc + sh
            kv = acc * vb[rows, b0 * BLK:(b0 + NH) * BLK].astype(F32)
            parts += [kv[:, a * BLK:(a + 1) * BLK] for a in range(NH)]
        return jnp.concatenate(parts, axis=0).astype(BF16)

    def conv_fwd(r0, nrows, b0, kv, tokens=None):
        first = b0 == 0
        hs = hb[pl.ds(r0, nrows), b0 * BLK:(b0 + NH) * BLK]
        hst = jnp.concatenate([hs[s:s + 16, a * BLK:(a + 1) * BLK]
                               for s in range(0, nrows, 16) for a in range(NH)], axis=0)
        if tokens:
            hst = _gated(hst, tokens)
        hf = _dot(hst, ftb[...])
        uf = _dot(kv, ftb[...])
        for gg in range(nrows // 8):
            r8 = pl.ds(r0 + gg * 8, 8)
            zp = None if first else hraw[r8, :]
            us, hs = [], []
            for a in range(NH):
                base = (gg // 2) * 16 * NH + a * 16 + (gg % 2) * 8
                z = uf[base:base + 8, :]
                ur, ui = z[:, :BLK], z[:, BLK:]
                us.append((ur + ui, ur, ui))
                z = hf[base:base + 8, :]
                if zp is None:
                    c = z[:, :BLK] + par[4, r8, :]
                    d = z[:, BLK:]
                else:
                    c = z[:, :BLK] - zp[:, BLK:]
                    d = z[:, BLK:] + zp[:, :BLK]
                hs.append((c, d - c, c + d))
                zp = z
            for p in range(3):
                up[p, b0:b0 + NH, r8, :] = jnp.stack([t[p] for t in us])
                hp[p, b0:b0 + NH, r8, :] = jnp.stack([t[p] for t in hs])
            if first:
                hraw[r8, :] = zp

    def conv_pairs(r0, b0, tokens=None):
        b1 = b0 + NH
        ks = []
        for p in range(3):
            kp = []
            for gg in range(2):
                r8 = pl.ds(r0 + gg * 8, 8)
                uu = up[p, :b1, r8, :]
                hh = hp[p, :b1, r8, :]
                ka = []
                for a in range(b0, b1):
                    acc = hh[0] * uu[a]
                    for j in range(1, a + 1):
                        acc = acc + hh[j] * uu[a - j]
                    ka.append(acc)
                kp.append(ka)
                if tokens is not None:
                    tokens.append(_token(ka))
            ks.append([jnp.concatenate([kp[0][a], kp[1][a]], axis=0) for a in range(NH)])
        return [jnp.concatenate([ks[0][a] - ks[2][a], ks[0][a] + ks[1][a]], axis=1)
                for a in range(NH)]

    def conv_inv(r0, parts, b0):
        ns = len(parts) // NH
        for tt in range(NH // TB):
            lhs = jnp.concatenate(
                [parts[s * NH + tt * TB + a] for s in range(ns) for a in range(TB)], axis=0)
            yt = _dot(lhs.astype(BF16), gib[...])
            cols = [jnp.concatenate(
                [yt[(s * TB + a) * 16:(s * TB + a + 1) * 16, :] for s in range(ns)], axis=0)
                for a in range(TB)]
            y_s[b0 // TB + tt, pl.ds(r0, ns * 16), :] = jnp.concatenate(cols, axis=1)

    def gate_layer(t, stats, pace=None):
        m, rs = stats
        st = _Stats(4)
        for r in range(0, D, 8):
            if r % 16 == 0:
                mb = _after(jnp.broadcast_to(m, (8, TM)), _tick(pace, r // 16, D // 16))
            x = x_s[t, r:r + 8, :]
            x1 = x + (x - mb) * rs * y_s[t, r:r + 8, :]
            x_s[t, r:r + 8, :] = x1
            st.add(x1)
        return st.finish()

    def ffn_operands(t, stats, pace=None):
        m, rs = stats
        rs = rs * XN_SCALE
        for r in range(0, KH, 16):
            mb = _after(jnp.broadcast_to(m, (8, TM)), _tick(pace, r // 16, KH // 16))
            mb = jnp.concatenate([mb, mb], axis=0)
            hi = (x_s[t, r:r + 16, :] - mb) * rs
            if KH + r < D:
                lo = (x_s[t, KH + r:KH + r + 16, :] - mb) * rs
            else:
                lo = jnp.zeros((16, TM), F32)
            for kk, b in enumerate(_b_combos(hi[:, :TH], hi[:, TH:], lo[:, :TH], lo[:, TH:])):
                bs[kk, r:r + 16, :] = b.astype(BF16)

    def head(before=None, after=None, r0=0, nr=FH):
        def prod(i, kk):
            tokens = before(i) if before is not None else None
            u = pltpu.bitcast(sg[kk, r0:r0 + nr, :], BF16)
            lhs = _gated(u, tokens, PAIR_SKIPS[i] if nr == FH else 0) if tokens else u
            m = _dot(lhs, bs[kk])
            if after is not None:
                after(i)
            return m

        m4 = prod(0, 3)
        m2 = prod(1, 1)
        hc[0, r0:r0 + nr, :] = _geglu(m2 + m4)
        m5 = prod(2, 4)
        m3 = prod(3, 2)
        hc[1, r0:r0 + nr, :] = _geglu(m3 + m5)
        m1 = prod(4, 0)
        ec[0, 2 * r0:2 * (r0 + nr), :] = (m4 - m5) + m1
        ec[1, 2 * r0:2 * (r0 + nr), :] = (m3 - m2) + m1

    init_state = {}

    def init_tile(t, tokens=None, lo=0, hi=D):
        if lo == 0:
            init_state['st'] = _Stats(4 if tokens is None else 1)
        st = init_state['st']
        for r in range(lo, hi, 16):
            x = qb[t, r:r + 16, :].astype(F32)
            x_s[t, r:r + 16, :] = x
            st.add(x[:8])
            st.add(x[8:])
            if tokens is not None and r % 32 == 16:
                e = st.s1[0] + st.s2[0]
                tokens.append(_token([e[:, j * BLK:(j + 1) * BLK] for j in range(TB)]))
        if hi < D:
            return None
        m, rs = st.finish()
        st0[t, 0:1, :] = m
        st0[t, 1:2, :] = rs
        return m, rs

    def tail(mid=None, after=None):
        def prod(i, kk, rhs):
            lhs = wdb[:DH, :FH] if kk == 2 else wdb[DH:, FH:] if kk == 3 else sd[kk]
            d = _dot(lhs, rhs.astype(BF16))
            if after is not None:
                after(i, d)
            return d

        m7 = _dot(pltpu.bitcast(sg[6], BF16), bs[6])
        h11 = _geglu(ec[0] + m7)
        m6 = _dot(pltpu.bitcast(sg[5], BF16), bs[5])
        h22 = _geglu(ec[1] + m6)
        if mid is not None:
            mid(m7, m6)
        h21, h12 = hc[0], hc[1]
        d2 = prod(0, 1, h11)
        d4 = prod(1, 3, h21 - h11)
        d6 = prod(2, 5, h11 + h12)
        d5 = prod(3, 4, h22)
        d1 = prod(4, 0, h11 + h22)
        d3 = prod(5, 2, h12 - h22)
        return d1, d2, d3, d4, d5, d6, lambda: prod(6, 6, h21 + h22)

    def residual(t, d):
        d1, d2, d3, d4, d5, d6, d7 = d
        d7 = d7()
        st = _Stats()
        for r in list(range(DH, D, 16)) + list(range(0, DH, 16)):
            if r < DH:
                q = slice(r, r + 16)
                f = jnp.concatenate([(d4[q] - d5[q]) + d1[q] + d7[q], d3[q] + d5[q]], axis=1)
            else:
                q = slice(r - DH, r - DH + 16)
                f = jnp.concatenate([d2[q] + d4[q], (d6[q] - d2[q]) + d1[q] + d3[q]], axis=1)
            xo = x_s[t, r:r + 16, :] + f
            ob[t, r:r + 16, :] = xo.astype(BF16)
            x_s[t, r:r + 16, :] = xo
            st.add(xo[:8])
            st.add(xo[8:])
        m, rs = st.finish()
        st0[t, 0:1, :] = m
        st0[t, 1:2, :] = rs

    def residual_last(d):
        t = NT - 1
        d1, d2, d3, d4, d5, d6, d7 = d
        ob[t, DH:, :] = (x_s[t, DH:, :] + jnp.concatenate(
            [d2 + d4, (d6 - d2) + d1 + d3], axis=1)).astype(BF16)
        ob[t, :DH, TH:] = (x_s[t, :DH, TH:] + (d3 + d5)).astype(BF16)
        e = x_s[t, :DH, :TH] + ((d4 - d5) + d1)
        d7 = d7()
        last_copy(0).start()
        last_copy(1).start()
        ob[t, :DH, :TH] = (e + d7).astype(BF16)
        last_copy(2).start()

    def prep_gate_up(c, tokens=None):
        combos = []
        for wbuf in (wgb, wub):
            blocks = []
            for half in range(2):
                t = wbuf[:, half * FH + c * BLK: half * FH + (c + 1) * BLK].astype(F32).T
                blocks.append(t[:, :KH])
                blocks.append(jnp.concatenate([t[:, KH:], jnp.zeros((BLK, 2 * KH - D), F32)],
                                              axis=1))
            combos.append(_a_combos(*blocks))
            if tokens is not None:
                e = combos[-1][0] + combos[-1][5]
                for r in range(0, BLK, 32):
                    tokens.append(_token([e[r + i:r + i + 8, j:j + BLK]
                                          for i in range(0, 32, 8) for j in range(0, KH, BLK)]))
        for kk in range(7):
            a = jnp.concatenate([combos[w][kk][16 * i:16 * i + 16]
                                 for i in range(BLK // 16) for w in range(2)], axis=0)
            sg[kk, c * BLK:(c + 1) * BLK, :] = pltpu.bitcast(a.astype(BF16), U32)

    def prep_down(lo, hi):
        tokens = []
        for r in range(lo, hi, 16):
            a11, a21 = (wdb[o + r:o + r + 16, :FH].astype(F32) for o in (0, DH))
            a12, a22 = (wdb[o + r:o + r + 16, FH:].astype(F32) for o in (0, DH))
            cs = _a_combos(a11, a12, a21, a22)
            for kk, a in enumerate(cs):
                if kk not in (2, 3):
                    sd[kk, r:r + 16, :] = a.astype(BF16)
            e = cs[0][:8] + cs[5][8:]
            tokens.append(_token([e[:, j * BLK:(j + 1) * BLK] for j in range(FH // BLK)]))
        return tokens

    parts = []
    for g in range(NC + 1):
        wait(c1_copies(g) if g < NC else [q_copy(0)])
        done, parts, tokens = parts, [], []
        if g > 0:
            for s in range(RC // 16):
                parts += conv_pairs((g - 1) * RC + s * 16, 0, tokens if g < NC else None)
        if g > 1:
            early, tokens = tokens[:N_EARLY], tokens[N_EARLY:]
            for n, z in enumerate(early):
                i = ((n // 2 + 1) * (RC // 16) // (N_EARLY // 2) - 1) * NH + (n % 2) * TB + TB - 1
                p = done[i]
                top = jnp.concatenate(
                    [p[:8, :BLK] + z.astype(jnp.int32).astype(F32), p[:8, BLK:]], axis=1)
                done[i] = jnp.concatenate([top, p[8:]], axis=0)
            conv_inv((g - 2) * RC, done, 0)
        if g < NC:
            conv_fwd(g * RC, RC, 0, conv_kv(g * RC, RC, 0), tokens)
    conv_inv((NC - 1) * RC, parts, 0)
    st = gate_layer(0, init_tile(0))
    wait(w_copies(0) + w_copies(1))
    ffn_operands(0, st)
    prep_gate_up(0)
    prep_gate_up(1)

    def prep_hook(chunks, wait_at):
        def before(i):
            tokens = []
            if i == wait_at:
                wait([c for g in chunks.values() for c in w_copies(g)])
            if i in chunks:
                prep_gate_up(chunks[i], tokens)
            return tokens
        return before

    def down_hook(i):
        tokens = []
        if i == 1:
            wait([wd_copy, q_copy(1)])
        if i > 0:
            tokens = prep_down((0, 48, 128, 176)[i - 1], (48, 128, 176, DH)[i - 1])
        if i in (2, 4):
            extra = []
            init_tile(1, extra, (i - 2) * DH // 2, i * DH // 2)
            tokens = [z for pair in zip(extra, tokens) for z in pair] + extra[len(tokens):]
        return tokens

    head(prep_hook({2: 2, 4: 3}, 2), None, 0, 2 * BLK)
    head(prep_hook({0: 4, 2: 5, 4: 6}, 0), None, 2 * BLK, 2 * BLK)
    head(down_hook, None, 4 * BLK, 3 * BLK)

    def tile_of(k):
        return 2 * (k // 4) + k % 2

    def step(k, with_conv):
        t_nxt = tile_of(k + 1)
        r0 = pl.multiple_of(k * R2_STRIDE, 16)
        box = {'d': []}

        def mid(m7, m6):
            st = (st0[t_nxt, 0:1, :], st0[t_nxt, 1:2, :])
            box['st'] = gate_layer(t_nxt, st, m7)
            if with_conv:
                box['kv'] = conv_kv(r0, R2, NH, m6)
            else:
                ffn_operands(t_nxt, box['st'], m6)

        def after_down(i, d):
            box['d'].append(d)
            if i == 2:
                ffn_operands(t_nxt, box['st'], jnp.concatenate(box['d'], axis=0))
                conv_fwd(r0, R2, NH, box['kv'])

        def before(i):
            tokens = []
            box['parts'] = []
            if i < len(PAIR_GROUPS):
                for s in range(PAIR_GROUPS[i]):
                    box['parts'] += conv_pairs(r0 + (sum(PAIR_GROUPS[:i]) + s) * 16, NH, tokens)
            else:
                init_tile(jnp.minimum(k + 2, NT - 1), tokens)
            return tokens

        def after(i):
            if box['parts']:
                conv_inv(r0 + sum(PAIR_GROUPS[:i]) * 16, box['parts'], NH)

        residual(tile_of(k), tail(mid, after_down if with_conv else None))
        if with_conv:
            head(before, after)
        else:
            head()

    def loop1(k, carry):
        for j in range(3):
            @pl.when(k == j)
            def _():
                wait(c2_copies(j))
        step(k, True)
        return carry

    def loop2(k, carry):
        step(k, False)
        for kk, t in ((3, 1), (6, 2)):
            @pl.when(k == kk)
            def _():
                o_copy(t).start()
        return carry

    lax.fori_loop(0, 3, loop1, 0)
    o_copy(0).start()
    lax.fori_loop(3, 7, loop2, 0)
    residual_last(tail())
    wait([o_copy(t) for t in range(NT - 1)] + [last_copy(n) for n in range(3)])


@jax.jit
def pallas_interleave_layers__ssm_conv_h3__geglu_ffn__prompt_kernel(A_q, A_k, A_v, A_shift_k, A_ssm_k, A_ssm_D, B_x, B_w_gate, B_w_up, B_w_down):
    ft, gi = _dft_consts()
    anyspec = pl.BlockSpec(memory_space=pl.ANY)
    vm = pltpu.VMEM
    out_t = pl.pallas_call(
        _kernel,
        in_specs=[anyspec] * 11,
        out_specs=anyspec,
        out_shape=jax.ShapeDtypeStruct((D, S), BF16),
        scratch_shapes=[
            vm((NT, D, TM), BF16), vm((D, S), BF16), vm((D, S), BF16), vm((D, S), BF16),
            vm((4, D), BF16), vm((D,), BF16),
            vm((D, F), BF16), vm((D, F), BF16), vm((D, F), BF16),
            vm((BLK, 2 * BLK), BF16), vm((2 * BLK, BLK), BF16),
            vm((7, F // 2, KH), U32), vm((7, DH, FH), BF16),
            vm((5, D, BLK), F32),
            vm((3, NB, D, BLK), F32), vm((3, NB, D, BLK), F32), vm((D, 2 * BLK), F32),
            vm((NT, D, TM), F32), vm((NT, D, TM), F32), vm((NT, 8, TM), F32),
            vm((7, KH, TH), BF16), vm((2, F, TH), F32), vm((2, FH, TH), F32),
            vm((NT, D, TM), BF16),
            pltpu.SemaphoreType.DMA((NUM_SEMS,)), pltpu.SemaphoreType.REGULAR,
        ],
        compiler_params=pltpu.CompilerParams(vmem_limit_bytes=110 * 1024 * 1024),
    )(A_q[0].T, A_k[0].T, A_v[0].T, A_shift_k.T, A_ssm_k, A_ssm_D,
      B_w_gate, B_w_up, B_w_down.T, ft, gi)
    return out_t.T[None]
```

```python
import numpy as np
import jax
import jax.numpy as jnp
from jax import lax
import jax.experimental.pallas as pl
import jax.experimental.pallas.tpu as pltpu

S, D, F = 2048, 448, 1792
BLK = 128
NB = S // BLK
NH = NB // 2
SH = S // 2
TM = 512
TB = TM // BLK
TH = TM // 2
NT = S // TM
FH = F // 2
DH = D // 2
KH = 256
NC = 7
RC = D // NC
R2 = 160
R2_STRIDE = 144
C2_ROWS = ((0, 160), (160, 144), (304, 144))
PAIR_GROUPS = (3, 2, 3, 2)
PAIR_SKIPS = (384, 192, 192, 192, 0)
PREP_SKIP = 128
N_EARLY = 8
SEM_C2 = NC
SEM_W01, SEM_W23, SEM_W46, SEM_Q0, SEM_WD, SEM_SMALL, SEM_OUT = (NC + 3 + i for i in range(7))
NUM_SEMS = NC + 10
EPS = 1e-5
HUGE = 3.0e38
F32 = jnp.float32
BF16 = jnp.bfloat16
U32 = jnp.uint32
XN_SCALE = float(np.sqrt(0.5))
GELU_C0 = float(np.sqrt(2.0 / np.pi)) / XN_SCALE
GELU_C1 = float(np.sqrt(2.0 / np.pi)) * 0.044715 / XN_SCALE ** 3


def _dft_consts():
    n = np.arange(BLK)[:, None]
    m = np.arange(BLK)[None, :]
    ang = np.pi * (((4 * m + 1) * n) % 512) / 256.0
    ft = np.concatenate([np.cos(ang), -np.sin(ang)], axis=1)
    gi = ft.T / BLK
    return jnp.asarray(ft, BF16), jnp.asarray(gi, BF16)


class _Stats:
    def __init__(self, ways=1):
        self.c = None
        self.n = 0
        self.s1 = [None] * ways
        self.s2 = [None] * ways

    def add(self, x):
        if self.c is None:
            self.c = x[0:1, :]
        xs = x - self.c
        w = self.n % len(self.s1)
        self.n += 1
        self.s1[w] = xs if self.s1[w] is None else self.s1[w] + xs
        self.s2[w] = xs * xs if self.s2[w] is None else self.s2[w] + xs * xs

    def finish(self):
        def tree(v):
            while len(v) > 1:
                v = [v[i] + v[i + 1] for i in range(0, len(v), 2)]
            return v[0]
        m = jnp.sum(tree(self.s1), axis=0, keepdims=True) * (1.0 / D)
        v = jnp.sum(tree(self.s2), axis=0, keepdims=True) * (1.0 / D) - m * m
        return self.c + m, lax.rsqrt(jnp.maximum(v, 0.0) + EPS)


def _a_combos(a11, a12, a21, a22):
    return [a11 + a22, a21 + a22, a11, a22, a11 + a12, a21 - a11, a12 - a22]


def _b_combos(b11, b12, b21, b22):
    return [b11 + b22, b11, b12 - b22, b21 - b11, b22, b11 + b12, b21 + b22]


def _geglu(c):
    n = c.shape[0] // 32
    g = jnp.concatenate([c[32 * i:32 * i + 16] for i in range(n)], axis=0)
    u = jnp.concatenate([c[32 * i + 16:32 * i + 32] for i in range(n)], axis=0)
    t = jnp.tanh(g * (GELU_C0 + GELU_C1 * (g * g)))
    gu = g * u
    return gu + gu * t


def _dot(a, b):
    return jnp.dot(a, b, preferred_element_type=F32)


def _tick(pace, i, n):
    if pace is None:
        return None
    r = (i * pace.shape[0] // n) // 8 * 8
    return jnp.where(pace[r:r + 8, :BLK] > HUGE, 1.0, 0.0)


def _after(x, z):
    if z is None:
        return x
    return x + jnp.tile(z, (x.shape[0] // 8, x.shape[1] // BLK))


def _token(vals):
    acc = vals[0]
    for v in vals[1:]:
        acc = acc + v
    return jnp.where(acc > HUGE, jnp.uint32(1), jnp.uint32(0))


def _gated(u, tokens, skip=0):
    n = len(tokens)
    pieces, prev = [], 0
    for i, z in enumerate(tokens):
        p = (skip + (i + 1) * (u.shape[0] - skip) // n) // 16 * 16 - 16
        seg = u[p:p + 16]
        pieces += [u[prev:p]] if p > prev else []
        first = pltpu.bitcast(pltpu.bitcast(seg[:, :BLK], U32) | z, BF16)
        pieces.append(jnp.concatenate([first, seg[:, BLK:]], axis=1) if u.shape[1] > BLK else first)
        prev = p + 16
    if prev < u.shape[0]:
        pieces.append(u[prev:])
    return jnp.concatenate(pieces, axis=0)


def _kernel(q_hbm, k_hbm, v_hbm, sk_hbm, h_hbm, d_hbm, wg_hbm, wu_hbm, wd_hbm, ft_hbm, gi_hbm,
            o_hbm,
            qb, kb, vb, hb, skb, db, wgb, wub, wdb, ftb, gib,
            sg, sd, par, up, hp, hraw, y_s, x_s, st0, bs, ec, hc, ob,
            sems, sem_f):
    kvh = ((k_hbm, kb), (v_hbm, vb), (h_hbm, hb))

    def fence():
        pl.semaphore_signal(sem_f, 1)
        pl.semaphore_wait(sem_f, 1)

    def c1_copies(g):
        rows, cols = pl.ds(g * RC, RC), pl.ds(0, SH)
        return [pltpu.make_async_copy(src.at[rows, cols], dst.at[rows, cols], sems.at[g])
                for src, dst in kvh]

    def c2_copies(j):
        rows, cols = pl.ds(*C2_ROWS[j]), pl.ds(SH, SH)
        cs = [pltpu.make_async_copy(src.at[rows, cols], dst.at[rows, cols], sems.at[SEM_C2 + j])
              for src, dst in kvh]
        return cs + ([q_copy(2 + j)] if j < 2 else [])

    def w_copies(g):
        sem = sems.at[(SEM_W01, SEM_W01, SEM_W23, SEM_W23, SEM_W46, SEM_W46, SEM_W46)[g]]
        cs = []
        for src, dst in ((wg_hbm, wgb), (wu_hbm, wub)):
            for half in range(2):
                cols = pl.ds(half * FH + g * BLK, BLK)
                cs.append(pltpu.make_async_copy(src.at[:, cols], dst.at[:, cols], sem))
        return cs

    def q_copy(t):
        sem = sems.at[(SEM_Q0, SEM_WD, SEM_C2, SEM_C2 + 1)[t]]
        return pltpu.make_async_copy(q_hbm.at[:, pl.ds(t * TM, TM)], qb.at[t], sem)

    wd_copy = pltpu.make_async_copy(wd_hbm, wdb, sems.at[SEM_WD])

    def o_copy(t):
        return pltpu.make_async_copy(ob.at[t], o_hbm.at[:, pl.ds(t * TM, TM)], sems.at[SEM_OUT])

    def last_copy(n):
        rows, cols = ((pl.ds(DH, DH), pl.ds(0, TM)), (pl.ds(0, DH), pl.ds(TH, TH)),
                      (pl.ds(0, DH), pl.ds(0, TH)))[n]
        dst = pl.ds((NT - 1) * TM + cols.start, cols.size)
        return pltpu.make_async_copy(ob.at[NT - 1, rows, cols], o_hbm.at[rows, dst],
                                     sems.at[SEM_OUT])

    small = [pltpu.make_async_copy(s, d, sems.at[SEM_SMALL]) for s, d in
             ((sk_hbm, skb), (d_hbm, db), (ft_hbm, ftb), (gi_hbm, gib))]

    def wait(copies):
        for c in copies:
            c.wait()

    for group in ([small] + [c1_copies(g) for g in range(NC)] + [[q_copy(0)]]
                  + [w_copies(g) for g in range(NC)] + [[wd_copy], [q_copy(1)]]
                  + [c2_copies(j) for j in range(3)]):
        for c in group:
            c.start()
        fence()

    wait(small)
    sk = skb[...].astype(F32)
    for t in range(4):
        par[t] = jnp.broadcast_to(sk[t:t + 1, :], (BLK, D)).T
    par[4] = jnp.broadcast_to(db[...].astype(F32).reshape(1, D), (BLK, D)).T

    def conv_kv(r0, nrows, b0, pace=None):
        first = b0 == 0
        off = 0 if first else BLK
        parts = []
        for s in range(nrows // 16):
            rows = pl.ds(r0 + s * 16, 16)
            kf = _after(kb[rows, b0 * BLK - off:(b0 + NH) * BLK].astype(F32),
                        _tick(pace, s, nrows // 16))
            nw = NH + off // BLK
            acc = kf[:, off:] * jnp.tile(par[0, rows, :], (1, NH))
            for t in range(1, 4):
                sh = pltpu.roll(kf * jnp.tile(par[t, rows, :], (1, nw)), t, 1)[:, off:]
                if first:
                    lane = lax.broadcasted_iota(jnp.int32, (16, BLK), 1)
                    sh = jnp.concatenate([jnp.where(lane >= t, sh[:, :BLK], 0.0), sh[:, BLK:]],
                                         axis=1)
                acc = acc + sh
            kv = acc * vb[rows, b0 * BLK:(b0 + NH) * BLK].astype(F32)
            parts += [kv[:, a * BLK:(a + 1) * BLK] for a in range(NH)]
        return jnp.concatenate(parts, axis=0).astype(BF16)

    def conv_fwd(r0, nrows, b0, kv, tokens=None):
        first = b0 == 0
        hs = hb[pl.ds(r0, nrows), b0 * BLK:(b0 + NH) * BLK]
        hst = jnp.concatenate([hs[s:s + 16, a * BLK:(a + 1) * BLK]
                               for s in range(0, nrows, 16) for a in range(NH)], axis=0)
        if tokens:
            hst = _gated(hst, tokens)
        hf = _dot(hst, ftb[...])
        uf = _dot(kv, ftb[...])
        for gg in range(nrows // 8):
            r8 = pl.ds(r0 + gg * 8, 8)
            zp = None if first else hraw[r8, :]
            us, hs = [], []
            for a in range(NH):
                base = (gg // 2) * 16 * NH + a * 16 + (gg % 2) * 8
                z = uf[base:base + 8, :]
                ur, ui = z[:, :BLK], z[:, BLK:]
                us.append((ur + ui, ur, ui))
                z = hf[base:base + 8, :]
                if zp is None:
                    c = z[:, :BLK] + par[4, r8, :]
                    d = z[:, BLK:]
                else:
                    c = z[:, :BLK] - zp[:, BLK:]
                    d = z[:, BLK:] + zp[:, :BLK]
                hs.append((c, d - c, c + d))
                zp = z
            for p in range(3):
                up[p, b0:b0 + NH, r8, :] = jnp.stack([t[p] for t in us])
                hp[p, b0:b0 + NH, r8, :] = jnp.stack([t[p] for t in hs])
            if first:
                hraw[r8, :] = zp

    def conv_pairs(r0, b0, tokens=None):
        b1 = b0 + NH
        ks = []
        for p in range(3):
            kp = []
            for gg in range(2):
                r8 = pl.ds(r0 + gg * 8, 8)
                uu = up[p, :b1, r8, :]
                hh = hp[p, :b1, r8, :]
                ka = []
                for a in range(b0, b1):
                    acc = hh[0] * uu[a]
                    for j in range(1, a + 1):
                        acc = acc + hh[j] * uu[a - j]
                    ka.append(acc)
                kp.append(ka)
                if tokens is not None:
                    tokens.append(_token(ka))
            ks.append([jnp.concatenate([kp[0][a], kp[1][a]], axis=0) for a in range(NH)])
        return [jnp.concatenate([ks[0][a] - ks[2][a], ks[0][a] + ks[1][a]], axis=1)
                for a in range(NH)]

    def conv_inv(r0, parts, b0):
        ns = len(parts) // NH
        for tt in range(NH // TB):
            lhs = jnp.concatenate(
                [parts[s * NH + tt * TB + a] for s in range(ns) for a in range(TB)], axis=0)
            yt = _dot(lhs.astype(BF16), gib[...])
            cols = [jnp.concatenate(
                [yt[(s * TB + a) * 16:(s * TB + a + 1) * 16, :] for s in range(ns)], axis=0)
                for a in range(TB)]
            y_s[b0 // TB + tt, pl.ds(r0, ns * 16), :] = jnp.concatenate(cols, axis=1)

    def gate_layer(t, stats, pace=None):
        m, rs = stats
        st = _Stats(2)
        for r in range(0, D, 8):
            if r % 16 == 0:
                mb = _after(jnp.broadcast_to(m, (8, TM)), _tick(pace, r // 16, D // 16))
            x = x_s[t, r:r + 8, :]
            x1 = x + (x - mb) * rs * y_s[t, r:r + 8, :]
            x_s[t, r:r + 8, :] = x1
            st.add(x1)
        return st.finish()

    def ffn_operands(t, stats, pace=None):
        m, rs = stats
        rs = rs * XN_SCALE
        for r in range(0, KH, 16):
            mb = _after(jnp.broadcast_to(m, (8, TM)), _tick(pace, r // 16, KH // 16))
            mb = jnp.concatenate([mb, mb], axis=0)
            hi = (x_s[t, r:r + 16, :] - mb) * rs
            if KH + r < D:
                lo = (x_s[t, KH + r:KH + r + 16, :] - mb) * rs
            else:
                lo = jnp.zeros((16, TM), F32)
            for kk, b in enumerate(_b_combos(hi[:, :TH], hi[:, TH:], lo[:, :TH], lo[:, TH:])):
                bs[kk, r:r + 16, :] = b.astype(BF16)

    def head(before=None, after=None, r0=0, nr=FH):
        def prod(i, kk):
            tokens = before(i) if before is not None else None
            u = pltpu.bitcast(sg[kk, r0:r0 + nr, :], BF16)
            lhs = _gated(u, tokens, PAIR_SKIPS[i] if nr == FH else PREP_SKIP) if tokens else u
            m = _dot(lhs, bs[kk])
            if after is not None:
                after(i)
            return m

        m4 = prod(0, 3)
        m2 = prod(1, 1)
        hc[0, r0:r0 + nr, :] = _geglu(m2 + m4)
        m5 = prod(2, 4)
        m3 = prod(3, 2)
        hc[1, r0:r0 + nr, :] = _geglu(m3 + m5)
        m1 = prod(4, 0)
        ec[0, 2 * r0:2 * (r0 + nr), :] = (m4 - m5) + m1
        ec[1, 2 * r0:2 * (r0 + nr), :] = (m3 - m2) + m1

    init_state = {}

    def init_tile(t, tokens=None, lo=0, hi=D):
        if lo == 0:
            init_state['st'] = _Stats(4 if tokens is None else 1)
        st = init_state['st']
        for r in range(lo, hi, 16):
            x = qb[t, r:r + 16, :].astype(F32)
            x_s[t, r:r + 16, :] = x
            st.add(x[:8])
            st.add(x[8:])
            if tokens is not None and r % 32 == 16:
                e = st.s1[0] + st.s2[0]
                tokens.append(_token([e[:, j * BLK:(j + 1) * BLK] for j in range(TB)]))
        if hi < D:
            return None
        m, rs = st.finish()
        st0[t, 0:1, :] = m
        st0[t, 1:2, :] = rs
        return m, rs

    def tail(mid=None, after=None):
        def prod(i, kk, rhs):
            lhs = wdb[:DH, :FH] if kk == 2 else wdb[DH:, FH:] if kk == 3 else sd[kk]
            d = _dot(lhs, rhs.astype(BF16))
            if after is not None:
                after(i, d)
            return d

        m7 = _dot(pltpu.bitcast(sg[6], BF16), bs[6])
        h11 = _geglu(ec[0] + m7)
        m6 = _dot(pltpu.bitcast(sg[5], BF16), bs[5])
        h22 = _geglu(ec[1] + m6)
        if mid is not None:
            mid(m7, m6)
        h21, h12 = hc[0], hc[1]
        d2 = prod(0, 1, h11)
        d4 = prod(1, 3, h21 - h11)
        d6 = prod(2, 5, h11 + h12)
        d5 = prod(3, 4, h22)
        d1 = prod(4, 0, h11 + h22)
        d3 = prod(5, 2, h12 - h22)
        return d1, d2, d3, d4, d5, d6, lambda: prod(6, 6, h21 + h22)

    def residual(t, d):
        d1, d2, d3, d4, d5, d6, d7 = d
        d7 = d7()
        st = _Stats()
        for r in list(range(DH, D, 16)) + list(range(0, DH, 16)):
            if r < DH:
                q = slice(r, r + 16)
                f = jnp.concatenate([(d4[q] - d5[q]) + d1[q] + d7[q], d3[q] + d5[q]], axis=1)
            else:
                q = slice(r - DH, r - DH + 16)
                f = jnp.concatenate([d2[q] + d4[q], (d6[q] - d2[q]) + d1[q] + d3[q]], axis=1)
            xo = x_s[t, r:r + 16, :] + f
            ob[t, r:r + 16, :] = xo.astype(BF16)
            x_s[t, r:r + 16, :] = xo
            st.add(xo[:8])
            st.add(xo[8:])
        m, rs = st.finish()
        st0[t, 0:1, :] = m
        st0[t, 1:2, :] = rs

    def residual_last(d):
        t = NT - 1
        d1, d2, d3, d4, d5, d6, d7 = d
        ob[t, DH:, :] = (x_s[t, DH:, :] + jnp.concatenate(
            [d2 + d4, (d6 - d2) + d1 + d3], axis=1)).astype(BF16)
        ob[t, :DH, TH:] = (x_s[t, :DH, TH:] + (d3 + d5)).astype(BF16)
        e = x_s[t, :DH, :TH] + ((d4 - d5) + d1)
        d7 = d7()
        last_copy(0).start()
        last_copy(1).start()
        ob[t, :DH, :TH] = (e + d7).astype(BF16)
        last_copy(2).start()

    def prep_gate_up(c, tokens=None):
        combos = []
        for wbuf in (wgb, wub):
            blocks = []
            for half in range(2):
                t = wbuf[:, half * FH + c * BLK: half * FH + (c + 1) * BLK].astype(F32).T
                blocks.append(t[:, :KH])
                blocks.append(jnp.concatenate([t[:, KH:], jnp.zeros((BLK, 2 * KH - D), F32)],
                                              axis=1))
            combos.append(_a_combos(*blocks))
            if tokens is not None:
                e = combos[-1][0] + combos[-1][5]
                for r in range(0, BLK, 32):
                    tokens.append(_token([e[r + i:r + i + 8, j:j + BLK]
                                          for i in range(0, 32, 8) for j in range(0, KH, BLK)]))
        for kk in range(7):
            a = jnp.concatenate([combos[w][kk][16 * i:16 * i + 16]
                                 for i in range(BLK // 16) for w in range(2)], axis=0)
            sg[kk, c * BLK:(c + 1) * BLK, :] = pltpu.bitcast(a.astype(BF16), U32)

    def prep_down(lo, hi):
        tokens = []
        for r in range(lo, hi, 16):
            a11, a21 = (wdb[o + r:o + r + 16, :FH].astype(F32) for o in (0, DH))
            a12, a22 = (wdb[o + r:o + r + 16, FH:].astype(F32) for o in (0, DH))
            cs = _a_combos(a11, a12, a21, a22)
            for kk, a in enumerate(cs):
                if kk not in (2, 3):
                    sd[kk, r:r + 16, :] = a.astype(BF16)
            e = cs[0][:8] + cs[5][8:]
            tokens.append(_token([e[:, j * BLK:(j + 1) * BLK] for j in range(FH // BLK)]))
        return tokens

    parts = []
    for g in range(NC + 1):
        wait(c1_copies(g) if g < NC else [q_copy(0)])
        done, parts, tokens = parts, [], []
        if g > 0:
            for s in range(RC // 16):
                parts += conv_pairs((g - 1) * RC + s * 16, 0, tokens if g < NC else None)
        if g > 1:
            early, tokens = tokens[:N_EARLY], tokens[N_EARLY:]
            for n, z in enumerate(early):
                i = ((n // 2 + 1) * (RC // 16) // (N_EARLY // 2) - 1) * NH + (n % 2) * TB + TB - 1
                p = done[i]
                top = jnp.concatenate(
                    [p[:8, :BLK] + z.astype(jnp.int32).astype(F32), p[:8, BLK:]], axis=1)
                done[i] = jnp.concatenate([top, p[8:]], axis=0)
            conv_inv((g - 2) * RC, done, 0)
        if g < NC:
            conv_fwd(g * RC, RC, 0, conv_kv(g * RC, RC, 0), tokens)
    conv_inv((NC - 1) * RC, parts, 0)
    st = gate_layer(0, init_tile(0))
    wait(w_copies(0) + w_copies(1))
    ffn_operands(0, st)
    prep_gate_up(0)
    prep_gate_up(1)

    def prep_hook(chunks, wait_at):
        def before(i):
            tokens = []
            if i == wait_at:
                wait([c for g in chunks.values() for c in w_copies(g)])
            if i in chunks:
                prep_gate_up(chunks[i], tokens)
            return tokens
        return before

    def down_hook(i):
        tokens = []
        if i == 1:
            wait([wd_copy, q_copy(1)])
        if i > 0:
            tokens = prep_down((0, 48, 128, 176)[i - 1], (48, 128, 176, DH)[i - 1])
        if i in (2, 4):
            extra = []
            init_tile(1, extra, (i - 2) * DH // 2, i * DH // 2)
            tokens = [z for pair in zip(extra, tokens) for z in pair] + extra[len(tokens):]
        return tokens

    head(prep_hook({2: 2, 4: 3}, 2), None, 0, 2 * BLK)
    head(prep_hook({0: 4, 2: 5, 4: 6}, 0), None, 2 * BLK, 2 * BLK)
    head(down_hook, None, 4 * BLK, 3 * BLK)

    def tile_of(k):
        return 2 * (k // 4) + k % 2

    def step(k, with_conv):
        t_nxt = tile_of(k + 1)
        r0 = pl.multiple_of(k * R2_STRIDE, 16)
        box = {'d': []}

        def mid(m7, m6):
            st = (st0[t_nxt, 0:1, :], st0[t_nxt, 1:2, :])
            box['st'] = gate_layer(t_nxt, st, m7)
            if with_conv:
                box['kv'] = conv_kv(r0, R2, NH, m6)
            else:
                ffn_operands(t_nxt, box['st'], m6)

        def after_down(i, d):
            box['d'].append(d)
            if i == 2:
                ffn_operands(t_nxt, box['st'], jnp.concatenate(box['d'], axis=0))
                conv_fwd(r0, R2, NH, box['kv'])

        def before(i):
            tokens = []
            box['parts'] = []
            if i < len(PAIR_GROUPS):
                for s in range(PAIR_GROUPS[i]):
                    box['parts'] += conv_pairs(r0 + (sum(PAIR_GROUPS[:i]) + s) * 16, NH, tokens)
            else:
                init_tile(jnp.minimum(k + 2, NT - 1), tokens)
            return tokens

        def after(i):
            if box['parts']:
                conv_inv(r0 + sum(PAIR_GROUPS[:i]) * 16, box['parts'], NH)

        residual(tile_of(k), tail(mid, after_down if with_conv else None))
        if with_conv:
            head(before, after)
        else:
            head()

    def loop1(k, carry):
        for j in range(3):
            @pl.when(k == j)
            def _():
                wait(c2_copies(j))
        step(k, True)
        return carry

    def loop2(k, carry):
        step(k, False)
        for kk, t in ((3, 1), (6, 2)):
            @pl.when(k == kk)
            def _():
                o_copy(t).start()
        return carry

    lax.fori_loop(0, 3, loop1, 0)
    o_copy(0).start()
    lax.fori_loop(3, 7, loop2, 0)
    residual_last(tail())
    wait([o_copy(t) for t in range(NT - 1)] + [last_copy(n) for n in range(3)])


@jax.jit
def pallas_interleave_layers__ssm_conv_h3__geglu_ffn__prompt_kernel(
    A_q: jax.Array,
    A_k: jax.Array,
    A_v: jax.Array,
    A_shift_k: jax.Array,
    A_ssm_k: jax.Array,
    A_ssm_D: jax.Array,
    B_x: jax.Array,
    B_w_gate: jax.Array,
    B_w_up: jax.Array,
    B_w_down: jax.Array,
):
    ft, gi = _dft_consts()
    anyspec = pl.BlockSpec(memory_space=pl.ANY)
    vm = pltpu.VMEM
    out_t = pl.pallas_call(
        _kernel,
        in_specs=[anyspec] * 11,
        out_specs=anyspec,
        out_shape=jax.ShapeDtypeStruct((D, S), BF16),
        scratch_shapes=[
            vm((NT, D, TM), BF16), vm((D, S), BF16), vm((D, S), BF16), vm((D, S), BF16),
            vm((4, D), BF16), vm((D,), BF16),
            vm((D, F), BF16), vm((D, F), BF16), vm((D, F), BF16),
            vm((BLK, 2 * BLK), BF16), vm((2 * BLK, BLK), BF16),
            vm((7, F // 2, KH), U32), vm((7, DH, FH), BF16),
            vm((5, D, BLK), F32),
            vm((3, NB, D, BLK), F32), vm((3, NB, D, BLK), F32), vm((D, 2 * BLK), F32),
            vm((NT, D, TM), F32), vm((NT, D, TM), F32), vm((NT, 8, TM), F32),
            vm((7, KH, TH), BF16), vm((2, F, TH), F32), vm((2, FH, TH), F32),
            vm((NT, D, TM), BF16),
            pltpu.SemaphoreType.DMA((NUM_SEMS,)), pltpu.SemaphoreType.REGULAR,
        ],
        compiler_params=pltpu.CompilerParams(vmem_limit_bytes=110 * 1024 * 1024),
    )(A_q[0].T, A_k[0].T, A_v[0].T, A_shift_k.T, A_ssm_k, A_ssm_D,
      B_w_gate, B_w_up, B_w_down.T, ft, gi)
    return out_t.T[None]
```
